```python
import os as _os
_os.environ.setdefault('JAX_PLATFORMS', 'cpu')
import jax
import jax.numpy as jnp

def _softmax(x, axis=-1):
    return jax.nn.softmax(x, axis=axis)

def _gelu(x):
    return jax.nn.gelu(x, approximate=True)

def _silu(x):
    return jax.nn.silu(x)

def _sigmoid(x):
    return jax.nn.sigmoid(x)

def _layernorm(x, axis=-1, eps=1e-05):
    m = jnp.mean(x, axis=axis, keepdims=True)
    v = jnp.var(x, axis=axis, keepdims=True)
    return (x - m) / jnp.sqrt(v + eps)

def _scatter_add(tgt, idx, src, axis=0):
    return tgt.at[idx].add(src)

def _segment_sum(src, seg, n):
    return jax.ops.segment_sum(src, seg, n)

class _Rng:

    def __init__(self, key):
        self._k = key

    def _next(self):
        self._k, sub = jax.random.split(self._k)
        return sub

    def normal(self, shape):
        return jax.random.normal(self._next(), shape, dtype=jnp.bfloat16)

    def randint(self, lo, hi, shape):
        return jax.random.randint(self._next(), shape, lo, hi, dtype=jnp.int32)

    def uniform(self, shape, lo=0.0, hi=1.0):
        return jax.random.uniform(self._next(), shape, jnp.bfloat16, lo, hi)

    def permutation(self, n):
        return jax.random.permutation(self._next(), n)
kernel_name = 'adaLN_cond__grouped_kv_mqa__mixer_gmlp__prompt'

def setup_inputs():
    _rng = _Rng(jax.random.key(int.from_bytes(__import__("os").urandom(4), "little")))
    _w = lambda a: (lambda t: t.astype(jnp.bfloat16) if jnp.issubdtype(t.dtype, jnp.floating) else t)(jnp.asarray(a))

    def _A_setup():
        B, S, D, H = (1, 2048, 512, 32)
        Dh = D // H
        return {'x': _w((lambda *s: _rng.normal(s) * 0.05)(B, S, D)), 'wq': _w((lambda *s: _rng.normal(s) * 0.05)(D, H * Dh)), 'wk': _w((lambda *s: _rng.normal(s) * 0.05)(D, Dh)), 'wv': _w((lambda *s: _rng.normal(s) * 0.05)(D, Dh)), 'wo': _w((lambda *s: _rng.normal(s) * 0.05)(H * Dh, D))}
    _A_in = _A_setup()

    def _B_setup():
        B, S, D, F = (1, 2048, 512, 1792)
        Fh = F // 2
        return {'x': _w((lambda *s: _rng.normal(s) * 0.05)(B, S, D)), 'w_in': _w((lambda *s: _rng.normal(s) * 0.4)(D, 2 * Fh)), 'w_sp': _w(0.01 * (lambda *s: _rng.normal(s) * 0.4)(S, S)), 'b_sp': _w(1.0 + 0.01 * (lambda *s: _rng.normal(s) * 0.05)(S)), 'w_out': _w((lambda *s: _rng.normal(s) * 0.05)(Fh, D))}
    _B_in = _B_setup()
    return {'A_x': _A_in['x'], 'A_wq': _A_in['wq'], 'A_wk': _A_in['wk'], 'A_wv': _A_in['wv'], 'A_wo': _A_in['wo'], 'B_x': _B_in['x'], 'B_w_in': _B_in['w_in'], 'B_w_sp': _B_in['w_sp'], 'B_b_sp': _B_in['b_sp'], 'B_w_out': _B_in['w_out'], 'c': _w((lambda *s: _rng.normal(s) * 0.05)(1, 512) * 8.0), 'w_mod': _w((lambda *s: _rng.normal(s) * 0.05)(512, 6 * 512) * 512 ** (-0.5) * 8.0)}

def reference(A_x, A_wq, A_wk, A_wv, A_wo, B_x, B_w_in, B_w_sp, B_b_sp, B_w_out, c, w_mod):

    def _A_ref(x, wq, wk, wv, wo):
        B, S, D = x.shape
        H = 32
        Dh = D // H
        q = (lambda x, *d: x.transpose(*d))((x @ wq).reshape(B, S, H, Dh), 0, 2, 1, 3)
        k = x @ wk
        v = x @ wv
        scores = jnp.einsum('bhqd,bkd->bhqk', q, k) * Dh ** (-0.5)
        p = _softmax(scores, axis=-1)
        o = jnp.einsum('bhqk,bkd->bhqd', p, v)
        return (lambda x, *d: x.transpose(*d))(o, 0, 2, 1, 3).reshape(B, S, H * Dh) @ wo

    def _B_ref(x, w_in, w_sp, b_sp, w_out):
        B, S, D = x.shape
        F = w_in.shape[-1]
        Fh = F // 2
        z = _gelu(jnp.einsum('bsd,df->bsf', x, w_in))
        z1 = z[..., :Fh].copy()
        z2 = _layernorm(z[..., Fh:], axis=-1)
        g = jnp.einsum('ts,bsf->btf', w_sp, z2) + b_sp[None, :, None]
        return jnp.einsum('bsf,fd->bsd', z1 * g, w_out)
    x = A_x
    mod = (_silu(c) @ w_mod).reshape(c.shape[0], 6, 1, -1)
    sa, ca, ga, sb, cb, gb = (mod[:, 0].copy(), mod[:, 1].copy(), mod[:, 2].copy(), mod[:, 3].copy(), mod[:, 4].copy(), mod[:, 5].copy())
    h = _layernorm(x, axis=-1) * (1 + ca) + sa
    x = x + ga * _A_ref(h, A_wq, A_wk, A_wv, A_wo)
    h = _layernorm(x, axis=-1) * (1 + cb) + sb
    x = x + gb * _B_ref(h, B_w_in, B_w_sp, B_b_sp, B_w_out)
    return x
```

```python
import math

import jax
import jax.numpy as jnp
from jax import lax
import jax.experimental.pallas as pl
import jax.experimental.pallas.tpu as pltpu

S = 2048
D = 512
H = 32
DH = 16
F = 1792
FH = F // 2
EPS = 1e-5

TQ = 512
KC = 128
NKC = S // KC
NQ = S // TQ
NSTAGE = NQ * H
U = 4
SKEW = 2
LAG_M = 2
LAG_L = 1

RB = 256
NRB = S // RB

QSCALE = (DH ** -0.5) * math.log2(math.e)

_F32 = jnp.float32
_BF16 = jnp.bfloat16


def _bits(x):
    return pltpu.bitcast(x, jnp.int32)


def _flt(x):
    return pltpu.bitcast(x, _F32)


def _ln(x):
    m = jnp.mean(x, axis=-1, keepdims=True)
    xc = x - m
    v = jnp.mean(xc * xc, axis=-1, keepdims=True)
    return xc * lax.rsqrt(v + EPS)


def _gelu(x):
    c = math.sqrt(2.0 / math.pi)
    inner = x * (c + (c * 0.044715) * (x * x))
    hx = 0.5 * x
    return hx + hx * jnp.tanh(inner)


def _dot(a, b):
    return jnp.dot(a, b, preferred_element_type=_F32)


def _dot_nt(a, b):
    return lax.dot_general(a, b, (((1,), (1,)), ((), ())), preferred_element_type=_F32)


def _dot_tn(a, b):
    return lax.dot_general(a, b, (((0,), (0,)), ((), ())), preferred_element_type=_F32)


def _kernel(x_hbm, wq_hbm, wk_hbm, wv_hbm, wo_hbm, win_hbm, wsp_hbm, bsp_hbm, wout_hbm,
            c_hbm, wmod_hbm, o_hbm,
            x_v, wq_v, wk_v, wv_v, wo_v, win_v, wsp_v, bsp_v, wout_v, c_v, wmod_v,
            mod_v, wqvt_v, k_v, vt_v, qt_v, ot_v, sa_v, sb_v, z_v,
            x1_v, z1_v, z2_v, out_v, sems, osems):
    copies = {
        "c": pltpu.make_async_copy(c_hbm, c_v, sems.at[0]),
        "wmod0": pltpu.make_async_copy(wmod_hbm.at[:, pl.ds(0, 2 * D)],
                                       wmod_v.at[:, pl.ds(0, 2 * D)], sems.at[1]),
        "wq": pltpu.make_async_copy(wq_hbm, wq_v, sems.at[2]),
        "wv": pltpu.make_async_copy(wv_hbm, wv_v, sems.at[3]),
        "wk": pltpu.make_async_copy(wk_hbm, wk_v, sems.at[4]),
        "x": pltpu.make_async_copy(x_hbm.at[0], x_v, sems.at[5]),
        "wmod1": pltpu.make_async_copy(wmod_hbm.at[:, pl.ds(2 * D, 4 * D)],
                                       wmod_v.at[:, pl.ds(2 * D, 4 * D)], sems.at[6]),
        "wo": pltpu.make_async_copy(wo_hbm, wo_v, sems.at[7]),
        "win": pltpu.make_async_copy(win_hbm, win_v, sems.at[8]),
        "wsp": pltpu.make_async_copy(wsp_hbm, wsp_v, sems.at[9]),
        "bsp": pltpu.make_async_copy(bsp_hbm, bsp_v, sems.at[10]),
        "wout": pltpu.make_async_copy(wout_hbm, wout_v, sems.at[11]),
    }
    for cp in copies.values():
        cp.start()

    z_v[...] = jnp.zeros(z_v.shape, z_v.dtype)

    copies["c"].wait()
    cf = c_v[...].astype(_F32)
    sc = (cf * jax.nn.sigmoid(cf)).astype(_BF16)
    sc8 = jnp.broadcast_to(sc, (16, D))
    copies["wmod0"].wait()
    mod_v[:, pl.ds(0, 2 * D)] = _dot(sc8, wmod_v[:, pl.ds(0, 2 * D)])[0:8]

    copies["wq"].wait()
    copies["wv"].wait()
    wqvt_v[pl.ds(0, D), :] = wq_v[...].astype(_F32).T.astype(_BF16)
    wv_pad = jnp.concatenate(
        [wv_v[...].astype(_F32), jnp.zeros((D, 128 - DH), _F32)], axis=1)
    wqvt_v[pl.ds(D, DH), :] = wv_pad.T[0:DH].astype(_BF16)
    copies["wk"].wait()
    copies["x"].wait()

    def qkv_body(r, carry):
        rows = pl.ds(pl.multiple_of(r * RB, RB), RB)
        xf = x_v[rows, :].astype(_F32)
        sa = mod_v[0:1, pl.ds(0, D)]
        ca = mod_v[0:1, pl.ds(D, D)]
        h = (_ln(xf) * (1.0 + ca) + sa).astype(_BF16)
        qvt = _dot_nt(wqvt_v[...], h)
        qt_v[:, rows] = (qvt[0:D] * QSCALE).astype(_BF16)
        vt_v[:, rows] = qvt[D:D + DH].astype(_BF16)
        k_v[rows, :] = _dot(h, wk_v[...]).astype(_BF16)
        return carry

    lax.fori_loop(0, NRB, qkv_body, 0)

    bufs = (sa_v, sb_v)

    def qslice(idx):
        qb = lax.shift_right_logical(idx, 5)
        h = lax.bitwise_and(idx, H - 1)
        return (pl.ds(pl.multiple_of(h * DH, DH), DH),
                pl.ds(pl.multiple_of(qb * TQ, TQ), TQ))

    def score_chunk(qt, buf, kc, m_acc):
        ks = pl.ds(kc * KC, KC)
        s = _dot(k_v[ks, :], qt)
        buf[ks, :] = s
        mm = jnp.max(s.reshape(KC // 8, 8, TQ), axis=0)
        return mm if m_acc is None else jnp.maximum(m_acc, mm)

    def pv_chunk(buf, kc, m_use, l_acc, o_acc):
        ks = pl.ds(kc * KC, KC)
        sc_ = buf[ks, :].reshape(KC // 8, 8, TQ)
        p = jnp.exp2(sc_ - m_use[None])
        for i in reversed(range(KC // 16)):
            a = p[2 * i] + p[2 * i + 1]
            l_acc = a if l_acc is None else l_acc + a
        pb = p.reshape(KC, TQ).astype(_BF16)
        o = _dot(vt_v[:, ks], pb)
        o_acc = o if o_acc is None else o + o_acc
        return l_acc, o_acc

    def finish(idx, l_acc, o_acc):
        l = jnp.sum(l_acc, axis=0, keepdims=True)
        r2, c2 = qslice(idx)
        ot_v[r2, c2] = (o_acc * (1.0 / l)).astype(ot_v.dtype)

    def full_max(m_acc):
        return jnp.broadcast_to(jnp.max(m_acc, axis=0, keepdims=True), (8, TQ))

    qt0 = qt_v[pl.ds(0, DH), pl.ds(0, TQ)]
    m_acc = None
    for kc in range(NKC):
        m_acc = score_chunk(qt0, bufs[0], kc, m_acc)
    m0 = full_max(m_acc)
    sb_v[pl.ds((NKC - SKEW) * KC, SKEW * KC), :] = jnp.zeros((SKEW * KC, TQ), _F32)

    def att_body(j, carry):
        m_prev, m_cur, l_acc, o_acc = carry
        i = U * j
        z = z_v[...]
        ms = {-1: m_prev, 0: m_cur}
        hist = []
        m_acc = None
        qt = None
        for t in range(U * NKC):
            u, kc = divmod(t, NKC)
            if kc == 0:
                r, c = qslice(jnp.minimum(i + u + 1, NSTAGE - 1))
                qt = qt_v[r, c]
                m_acc = None
            m_acc = score_chunk(qt, bufs[(u + 1) % 2], kc, m_acc)
            if kc == NKC - 1:
                ms[u + 1] = full_max(m_acc)
            u2, kc2 = divmod(t - SKEW, NKC)
            if kc2 == 0:
                l_acc = None
                o_acc = None
            m_use = ms[u2]
            dep = None
            if t >= LAG_M:
                dep = _bits(hist[t - LAG_M][0])
            if t >= LAG_L:
                hl = _bits(hist[t - LAG_L][1])
                dep = hl if dep is None else dep | hl
            if dep is not None:
                m_use = _flt(_bits(m_use) | (dep & z))
            l_acc, o_acc = pv_chunk(bufs[u2 % 2], kc2, m_use, l_acc, o_acc)
            hist.append((m_acc, l_acc))
            if kc2 == NKC - 1:
                finish(jnp.maximum(i + u2, 0), l_acc, o_acc)
        return ms[U - 1], ms[U], l_acc, o_acc

    zf = jnp.zeros((8, TQ), _F32)
    m_prev, _, l_acc, o_acc = lax.fori_loop(
        0, NSTAGE // U, att_body, (zf, m0, zf, jnp.zeros((DH, TQ), _F32)))
    for kc2 in range(NKC - SKEW, NKC):
        l_acc, o_acc = pv_chunk(bufs[(NSTAGE - 1) % 2], kc2, m_prev, l_acc, o_acc)
    finish(jnp.int32(NSTAGE - 1), l_acc, o_acc)

    copies["wmod1"].wait()
    mod_v[:, pl.ds(2 * D, 4 * D)] = _dot(sc8, wmod_v[:, pl.ds(2 * D, 4 * D)])[0:8]
    copies["wo"].wait()
    copies["win"].wait()

    def mid_body(r, carry):
        rows = pl.ds(pl.multiple_of(r * RB, RB), RB)
        ga = mod_v[0:1, pl.ds(2 * D, D)]
        sb = mod_v[0:1, pl.ds(3 * D, D)]
        cb = mod_v[0:1, pl.ds(4 * D, D)]
        o = ot_v[:, rows].T.astype(_BF16)
        a = _dot(o, wo_v[...])
        x1 = x_v[rows, :].astype(_F32) + ga * a
        x1_v[rows, :] = x1
        h2 = (_ln(x1) * (1.0 + cb) + sb).astype(_BF16)
        z1_v[rows, :] = _gelu(_dot(h2, win_v[:, pl.ds(0, FH)]))
        z2 = _gelu(_dot(h2, win_v[:, pl.ds(FH, FH)]))
        z2_v[rows, :] = _ln(z2).astype(_BF16)
        return carry

    lax.fori_loop(0, NRB, mid_body, 0)

    copies["wsp"].wait()
    copies["bsp"].wait()
    copies["wout"].wait()

    def out_copy(r, slot):
        rows = pl.ds(pl.multiple_of(r * RB, RB), RB)
        return pltpu.make_async_copy(out_v.at[slot], o_hbm.at[0, rows], osems.at[slot])

    def fin_body(r, carry):
        rows = pl.ds(pl.multiple_of(r * RB, RB), RB)
        slot = lax.bitwise_and(r, 1)
        gb = mod_v[0:1, pl.ds(5 * D, D)]
        brow = bsp_v[:, rows].astype(_F32)
        bcol = jnp.broadcast_to(brow, (128, RB)).T
        g = _dot(wsp_v[rows, :], z2_v[...])
        g = g + jnp.concatenate([bcol] * (FH // 128), axis=1)
        u = (z1_v[rows, :] * g).astype(_BF16)
        y = _dot(u, wout_v[...])
        res = (x1_v[rows, :] + gb * y).astype(_BF16)

        @pl.when(r >= 2)
        def _():
            out_copy(r - 2, slot).wait()

        out_v[slot] = res
        out_copy(r, slot).start()
        return carry

    lax.fori_loop(0, NRB, fin_body, 0)
    out_copy(NRB - 2, (NRB - 2) % 2).wait()
    out_copy(NRB - 1, (NRB - 1) % 2).wait()


@jax.jit
def pallas_adaLN_cond__grouped_kv_mqa__mixer_gmlp__prompt_kernel(
    A_x: jax.Array,
    A_wq: jax.Array,
    A_wk: jax.Array,
    A_wv: jax.Array,
    A_wo: jax.Array,
    B_x: jax.Array,
    B_w_in: jax.Array,
    B_w_sp: jax.Array,
    B_b_sp: jax.Array,
    B_w_out: jax.Array,
    c: jax.Array,
    w_mod: jax.Array,
):
    del B_x
    any_spec = pl.BlockSpec(memory_space=pl.ANY)
    scratch = [
        pltpu.VMEM((S, D), _BF16),
        pltpu.VMEM((D, D), _BF16),
        pltpu.VMEM((D, DH), _BF16),
        pltpu.VMEM((D, DH), _BF16),
        pltpu.VMEM((D, D), _BF16),
        pltpu.VMEM((D, F), _BF16),
        pltpu.VMEM((S, S), _BF16),
        pltpu.VMEM((1, S), _BF16),
        pltpu.VMEM((FH, D), _BF16),
        pltpu.VMEM((1, D), _BF16),
        pltpu.VMEM((D, 6 * D), _BF16),
        pltpu.VMEM((8, 6 * D), _F32),
        pltpu.VMEM((D + DH, D), _BF16),
        pltpu.VMEM((S, DH), _BF16),
        pltpu.VMEM((DH, S), _BF16),
        pltpu.VMEM((D, S), _BF16),
        pltpu.VMEM((D, S), _F32),
        pltpu.VMEM((S, TQ), _F32),
        pltpu.VMEM((S, TQ), _F32),
        pltpu.VMEM((8, TQ), jnp.int32),
        pltpu.VMEM((S, D), _F32),
        pltpu.VMEM((S, FH), _F32),
        pltpu.VMEM((S, FH), _BF16),
        pltpu.VMEM((2, RB, D), _BF16),
        pltpu.SemaphoreType.DMA((12,)),
        pltpu.SemaphoreType.DMA((2,)),
    ]
    return pl.pallas_call(
        _kernel,
        out_shape=jax.ShapeDtypeStruct((1, S, D), _BF16),
        in_specs=[any_spec] * 11,
        out_specs=any_spec,
        scratch_shapes=scratch,
        compiler_params=pltpu.CompilerParams(vmem_limit_bytes=100 * 1024 * 1024),
        name="adaln_mqa_gmlp",
    )(A_x, A_wq, A_wk, A_wv, A_wo, B_w_in, B_w_sp, B_b_sp.reshape(1, S), B_w_out, c, w_mod)
```

```python
import math

import jax
import jax.numpy as jnp
from jax import lax
import jax.experimental.pallas as pl
import jax.experimental.pallas.tpu as pltpu

S = 2048
D = 512
H = 32
DH = 16
F = 1792
FH = F // 2
EPS = 1e-5

TQ = 512
KC = 128
NKC = S // KC
NQ = S // TQ
NSTAGE = NQ * H
NL = TQ // 128
U = 16
DELTA = 1
LLAG = 10
GOFF = (8, 10, 12, 14)
L_LO = 2.0 ** -40
L_HI = 2.0 * S

RB = 256
NRB = S // RB
MU = 2
FU = 1

QSCALE = (DH ** -0.5) * math.log2(math.e)

_F32 = jnp.float32
_BF16 = jnp.bfloat16
_U32 = jnp.uint32


def _bits(x):
    return pltpu.bitcast(x, jnp.int32)


def _flt(x):
    return pltpu.bitcast(x, _F32)


def _ln(x):
    m = jnp.mean(x, axis=-1, keepdims=True)
    xc = x - m
    v = jnp.mean(xc * xc, axis=-1, keepdims=True)
    return xc * lax.rsqrt(v + EPS)


def _gelu(x):
    c = math.sqrt(2.0 / math.pi)
    inner = x * (c + (c * 0.044715) * (x * x))
    hx = 0.5 * x
    return hx + hx * jnp.tanh(inner)


def _dot(a, b):
    return jnp.dot(a, b, preferred_element_type=_F32)


def _dot_nt(a, b):
    return lax.dot_general(a, b, (((1,), (1,)), ((), ())), preferred_element_type=_F32)


def _dot_tn(a, b):
    return lax.dot_general(a, b, (((0,), (0,)), ((), ())), preferred_element_type=_F32)


def _kernel(x_hbm, wq_hbm, wk_hbm, wv_hbm, wo_hbm, win_hbm, wsp_hbm, bsp_hbm, wout_hbm,
            c_hbm, wmod_hbm, o_hbm,
            x_v, wq_v, wk_v, wv_v, wo_v, win_v, wsp_v, bsp_v, wout_v, c_v, wmod_v,
            mod_v, wt_v, k_v, vt_v, kb_v, qf_v, nm_v, qs_v, l_v, ot_v, z_v,
            x1_v, z1_v, z2_v, out_v, sems, xsems, osems):
    def x_copy(r):
        rows = pl.ds(r * RB, RB)
        return pltpu.make_async_copy(x_hbm.at[0, rows], x_v.at[rows], xsems.at[r])

    early = {
        "c": pltpu.make_async_copy(c_hbm, c_v, sems.at[0]),
        "wq": pltpu.make_async_copy(wq_hbm, wq_v, sems.at[2]),
        "wv": pltpu.make_async_copy(wv_hbm, wv_v, sems.at[3]),
        "wk": pltpu.make_async_copy(wk_hbm, wk_v, sems.at[4]),
        "wmod0": pltpu.make_async_copy(wmod_hbm.at[:, pl.ds(0, 2 * D)],
                                       wmod_v.at[:, pl.ds(0, 2 * D)], sems.at[1]),
    }
    late = {
        "wmod1": pltpu.make_async_copy(wmod_hbm.at[:, pl.ds(2 * D, 4 * D)],
                                       wmod_v.at[:, pl.ds(2 * D, 4 * D)], sems.at[6]),
        "wo": pltpu.make_async_copy(wo_hbm, wo_v, sems.at[7]),
        "win": pltpu.make_async_copy(win_hbm, win_v, sems.at[8]),
        "wsp": pltpu.make_async_copy(wsp_hbm, wsp_v, sems.at[9]),
        "bsp": pltpu.make_async_copy(bsp_hbm, bsp_v, sems.at[10]),
        "wout": pltpu.make_async_copy(wout_hbm, wout_v, sems.at[11]),
    }
    for cp in early.values():
        cp.start()
    for r in range(NRB):
        x_copy(r).start()

    z_v[...] = jnp.zeros(z_v.shape, z_v.dtype)

    early["wq"].wait()
    early["wv"].wait()
    early["wk"].wait()
    wt_v[pl.ds(0, D), :] = wq_v[...].astype(_F32).T.astype(_BF16)
    wvk = jnp.concatenate(
        [wv_v[...].astype(_F32), wk_v[...].astype(_F32),
         jnp.zeros((D, 128 - 2 * DH), _F32)], axis=1)
    wt_v[pl.ds(D, 2 * DH), :] = wvk.T[0:2 * DH].astype(_BF16)

    early["c"].wait()
    cf = c_v[...].astype(_F32)
    sc = (cf * jax.nn.sigmoid(cf)).astype(_BF16)
    sc8 = jnp.broadcast_to(sc, (16, D))
    early["wmod0"].wait()
    mod_v[:, pl.ds(0, 2 * D)] = _dot(sc8, wmod_v[:, pl.ds(0, 2 * D)])[0:8]

    sub = lax.broadcasted_iota(jnp.int32, (128 - DH, RB), 0)
    one_row = jnp.where(sub == 0, 1.0, 0.0)
    kmax2 = None
    for r in range(NRB):
        rows = pl.ds(r * RB, RB)
        x_copy(r).wait()
        xf = x_v[rows, :].astype(_F32)
        sa = mod_v[0:1, pl.ds(0, D)]
        ca = mod_v[0:1, pl.ds(D, D)]
        h = (_ln(xf) * (1.0 + ca) + sa).astype(_BF16)
        t = _dot_nt(wt_v[...], h)
        q = (t[0:D] * QSCALE).astype(_BF16).astype(_F32).reshape(H, DH, RB)
        qf_v[:, :, rows] = q
        nm_v[:, rows] = jnp.sum(q * q, axis=1)
        vt_v[:, rows] = pltpu.bitcast(t[D:D + DH].astype(_BF16), _U32)
        kt = t[D + DH:D + 2 * DH].astype(_BF16).astype(_F32)
        k2 = jnp.sum(kt * kt, axis=0, keepdims=True)
        kmax2 = k2 if kmax2 is None else jnp.maximum(kmax2, k2)
        kx = jnp.concatenate([kt, one_row], axis=0).T
        k_v[pl.ds(r * RB // 2, RB // 2), :] = pltpu.bitcast(
            kx[:, 0:2 * DH].astype(_BF16), _U32)
        for cc in range(RB // KC):
            kk = kx[cc * KC:cc * KC + 16]
            for d in range(DH):
                kb_v[r * (RB // KC) + cc, d] = jnp.broadcast_to(kk[:, d:d + 1], (16, 128))

    for cp in late.values():
        cp.start()

    kmax2 = jnp.max(kmax2, axis=1, keepdims=True)
    nm_v[...] = (jnp.sqrt(nm_v[...] * kmax2) * (-1.01)).astype(_BF16).astype(_F32)

    def stage_idx(idx):
        qb = lax.shift_right_logical(idx, 5)
        h = lax.bitwise_and(idx, H - 1)
        return h, pl.ds(pl.multiple_of(qb * TQ, TQ), TQ)

    T = U * NKC
    stream = [(t, b) for t in range(T) for b in range(7, 0, -1)]
    NS = len(stream)
    cuts = {}
    for t in range(T):
        cuts.setdefault(min(7 * (t + 2) + DELTA, NS), []).append(t)
    gates, inserts = {}, {}
    for t in range(T):
        u = t // NKC
        for jj in range(NL):
            g = 7 * t + GOFF[jj]
            ins = min(max(g - LLAG, 7 * NKC * u - 1), 7 * NKC * (u + 1) - 1)
            inserts.setdefault(ins, []).append((t, jj))
            if g < NS:
                gates[g] = (t, jj)

    def att_body(j, carry):
        never = z_v[...] != 0
        st = {}
        for u in range(U):
            h, c = stage_idx(U * j + u)
            st[u] = dict(o=None, l=[None] * NL, h=h, c=c, qt=None)
        tiles = {t: [None] * 8 for t in range(T)}
        vp, gval = {}, {}

        def stage_setup(u):
            s_ = st[u]
            if s_["qt"] is not None:
                return
            q = qf_v[s_["h"], :, s_["c"]]
            nm = jnp.broadcast_to(nm_v[pl.ds(s_["h"], 1), s_["c"]], (DH, TQ))
            s_["qt"] = jnp.concatenate([q.astype(_BF16), nm.astype(_BF16)], axis=0)
            qs_v[u, 0:DH] = q
            qs_v[u, DH:DH + 8] = nm[0:8]

        def ladd(u, jj, x):
            l = st[u]["l"]
            l[jj] = x if l[jj] is None else l[jj] + x

        def vpu_unit(t, jj):
            u, kc = divmod(t, NKC)
            stage_setup(u)
            ls = pl.ds(128 * jj, 128)
            acc = [qs_v[u, DH:DH + 8, ls]] * 2
            for d in range(DH):
                qd = jnp.broadcast_to(qs_v[u, pl.ds(d, 1), ls], (8, 128))
                for a in range(2):
                    acc[a] = acc[a] + kb_v[kc, d, pl.ds(8 * a, 8), :] * qd
            p = [jnp.exp2(x) for x in acc]
            vp[(t, jj)] = jnp.concatenate(p, axis=0)
            ladd(u, jj, p[0] + p[1])
            gval[(t, jj)] = st[u]["l"][jj]

        def pv(t):
            u, kc = divmod(t, NKC)
            vt = pltpu.bitcast(vt_v[:, pl.ds(kc * KC, KC)], _BF16)
            tiles[t][0] = jnp.concatenate([vp[(t, jj)] for jj in range(NL)], axis=1)
            pb = jnp.concatenate(tiles[t], axis=0).astype(_BF16)
            o = _dot(vt, pb)
            s_ = st[u]
            s_["o"] = o if s_["o"] is None else o + s_["o"]
            if kc == NKC - 1:
                l = jnp.sum(jnp.concatenate(s_["l"], axis=1), axis=0, keepdims=True)
                ot_v[s_["h"], :, s_["c"]] = s_["o"] * (1.0 / l)
                l_v[pl.ds(s_["h"], 1), s_["c"]] = l

        def flush(group):
            if not group:
                return
            u = group[0][1] // NKC
            stage_setup(u)
            kb = []
            for i_, t, b in group:
                k_ = k_v[pl.ds((t % NKC) * (KC // 2) + 8 * b, 8), :]
                if i_ in gates:
                    pu = pltpu.bitcast(gval[gates[i_]], _U32)
                    k_ = jnp.where(never, pu[:, 0:2 * DH], k_)
                kb.append(k_)
            kk = pltpu.bitcast(jnp.concatenate(kb, axis=0), _BF16)
            s = _dot(kk, st[u]["qt"])
            for g_, (i_, t, b) in enumerate(group):
                p = jnp.exp2(s[16 * g_:16 * g_ + 16])
                a = p[0:8] + p[8:16]
                for jj in range(NL):
                    ladd(u, jj, a[:, 128 * jj:128 * jj + 128])
                tiles[t][b] = p
                for key in inserts.get(i_, []):
                    vpu_unit(*key)

        for key in inserts.get(-1, []):
            vpu_unit(*key)
        group = []
        for i_, (t, b) in enumerate(stream):
            if i_ in cuts or i_ % (7 * NKC) == 0 or len(group) >= LLAG:
                flush(group)
                group = []
            for tt in cuts.get(i_, []):
                pv(tt)
            group.append((i_, t, b))
        flush(group)
        for tt in cuts[NS]:
            pv(tt)
        return carry

    lax.fori_loop(0, NSTAGE // U, att_body, 0)

    lall = l_v[...]
    ok = jnp.logical_and(lall >= L_LO, lall <= L_HI)
    nbad = jnp.sum(jnp.where(ok, 0.0, 1.0))

    @pl.when(nbad > 0.0)
    def _():
        def slow_stage(idx, carry):
            h, c = stage_idx(idx)
            qt = jnp.concatenate([qf_v[h, :, c].astype(_BF16),
                                  jnp.zeros((DH, TQ), _BF16)], axis=0)

            def scores(kc):
                kr = pl.ds(pl.multiple_of(kc * (KC // 2), KC // 2), KC // 2)
                return _dot(pltpu.bitcast(k_v[kr, :], _BF16), qt)

            def max_body(kc, m):
                return jnp.maximum(m, jnp.max(scores(kc), axis=0, keepdims=True))

            m = lax.fori_loop(0, NKC, max_body, jnp.full((1, TQ), -jnp.inf, _F32))

            def pv_body(kc, lo):
                l, o = lo
                p = jnp.exp2(scores(kc) - m)
                ks = pl.ds(pl.multiple_of(kc * KC, KC), KC)
                vt = pltpu.bitcast(vt_v[:, ks], _BF16)
                return (l + jnp.sum(p, axis=0, keepdims=True),
                        o + _dot(vt, p.astype(_BF16)))

            l, o = lax.fori_loop(0, NKC, pv_body,
                                 (jnp.zeros((1, TQ), _F32), jnp.zeros((DH, TQ), _F32)))
            ot_v[h, :, c] = o * (1.0 / l)
            return carry

        lax.fori_loop(0, NSTAGE, slow_stage, 0)

    late["wmod1"].wait()
    mod_v[:, pl.ds(2 * D, 4 * D)] = _dot(sc8, wmod_v[:, pl.ds(2 * D, 4 * D)])[0:8]
    late["wo"].wait()
    late["win"].wait()

    def mid_block(rows):
        ga = mod_v[0:1, pl.ds(2 * D, D)]
        sb = mod_v[0:1, pl.ds(3 * D, D)]
        cb = mod_v[0:1, pl.ds(4 * D, D)]
        o = ot_v[:, :, rows].reshape(D, RB).T.astype(_BF16)
        a = _dot(o, wo_v[...])
        x1 = x_v[rows, :].astype(_F32) + ga * a
        x1_v[rows, :] = x1
        h2 = (_ln(x1) * (1.0 + cb) + sb).astype(_BF16)
        z1_v[rows, :] = _gelu(_dot(h2, win_v[:, pl.ds(0, FH)]))
        z2 = _gelu(_dot(h2, win_v[:, pl.ds(FH, FH)]))
        z2_v[rows, :] = _ln(z2).astype(_BF16)

    def mid_body(r, carry):
        for e in range(MU):
            mid_block(pl.ds(pl.multiple_of((r * MU + e) * RB, RB), RB))
        return carry

    if MU == NRB:
        for r in range(NRB):
            mid_block(pl.ds(r * RB, RB))
    else:
        lax.fori_loop(0, NRB // MU, mid_body, 0)

    late["wsp"].wait()
    late["bsp"].wait()
    late["wout"].wait()

    def out_copy(r):
        rows = pl.ds(pl.multiple_of(r * RB, RB), RB)
        return pltpu.make_async_copy(out_v.at[rows], o_hbm.at[0, rows], osems.at[r])

    def fin_block(r):
        rows = pl.ds(pl.multiple_of(r * RB, RB), RB)
        gb = mod_v[0:1, pl.ds(5 * D, D)]
        brow = bsp_v[:, rows].astype(_F32)
        bcol = jnp.broadcast_to(brow, (128, RB)).T
        g = _dot(wsp_v[rows, :], z2_v[...])
        g = g + jnp.concatenate([bcol] * (FH // 128), axis=1)
        u = (z1_v[rows, :] * g).astype(_BF16)
        y = _dot(u, wout_v[...])
        out_v[rows, :] = (x1_v[rows, :] + gb * y).astype(_BF16)

    def fin_body(r, carry):
        for e in range(FU):
            fin_block(r * FU + e)
        for e in range(FU):
            out_copy(r * FU + e).start()
        return carry

    lax.fori_loop(0, NRB // FU, fin_body, 0)
    for r in range(NRB):
        out_copy(r).wait()


@jax.jit
def pallas_adaLN_cond__grouped_kv_mqa__mixer_gmlp__prompt_kernel(
    A_x: jax.Array,
    A_wq: jax.Array,
    A_wk: jax.Array,
    A_wv: jax.Array,
    A_wo: jax.Array,
    B_x: jax.Array,
    B_w_in: jax.Array,
    B_w_sp: jax.Array,
    B_b_sp: jax.Array,
    B_w_out: jax.Array,
    c: jax.Array,
    w_mod: jax.Array,
):
    del B_x
    any_spec = pl.BlockSpec(memory_space=pl.ANY)
    scratch = [
        pltpu.VMEM((S, D), _BF16),
        pltpu.VMEM((D, D), _BF16),
        pltpu.VMEM((D, DH), _BF16),
        pltpu.VMEM((D, DH), _BF16),
        pltpu.VMEM((D, D), _BF16),
        pltpu.VMEM((D, F), _BF16),
        pltpu.VMEM((S, S), _BF16),
        pltpu.VMEM((1, S), _BF16),
        pltpu.VMEM((FH, D), _BF16),
        pltpu.VMEM((1, D), _BF16),
        pltpu.VMEM((D, 6 * D), _BF16),
        pltpu.VMEM((8, 6 * D), _F32),
        pltpu.VMEM((D + 2 * DH, D), _BF16),
        pltpu.VMEM((S // 2, 2 * DH), _U32),
        pltpu.VMEM((DH // 2, S), _U32),
        pltpu.VMEM((NKC, DH, 16, 128), _F32),
        pltpu.VMEM((H, DH, S), _F32),
        pltpu.VMEM((H, S), _F32),
        pltpu.VMEM((U, DH + 8, TQ), _F32),
        pltpu.VMEM((H, S), _F32),
        pltpu.VMEM((H, DH, S), _F32),
        pltpu.VMEM((8, 2 * DH), jnp.int32),
        pltpu.VMEM((S, D), _F32),
        pltpu.VMEM((S, FH), _F32),
        pltpu.VMEM((S, FH), _BF16),
        pltpu.VMEM((S, D), _BF16),
        pltpu.SemaphoreType.DMA((12,)),
        pltpu.SemaphoreType.DMA((NRB,)),
        pltpu.SemaphoreType.DMA((NRB,)),
    ]
    return pl.pallas_call(
        _kernel,
        out_shape=jax.ShapeDtypeStruct((1, S, D), _BF16),
        in_specs=[any_spec] * 11,
        out_specs=any_spec,
        scratch_shapes=scratch,
        compiler_params=pltpu.CompilerParams(vmem_limit_bytes=100 * 1024 * 1024),
        name="adaln_mqa_gmlp",
    )(A_x, A_wq, A_wk, A_wv, A_wo, B_w_in, B_w_sp, B_b_sp.reshape(1, S), B_w_out, c, w_mod)
```

```python
import math

import jax
import jax.numpy as jnp
from jax import lax
import jax.experimental.pallas as pl
import jax.experimental.pallas.tpu as pltpu

S = 2048
D = 512
H = 32
DH = 16
F = 1792
FH = F // 2
EPS = 1e-5

TQ = 512
KC = 128
NKC = S // KC
NQ = S // TQ
NSTAGE = NQ * H
NL = TQ // 128
U = 16
DELTA = 1
LLAG = 10
GOFF = (8, 10, 12, 14)
L_LO = 2.0 ** -40
L_HI = 2.0 * S

RB = 256
NRB = S // RB
MU = 2
FU = 1

QSCALE = (DH ** -0.5) * math.log2(math.e)

_F32 = jnp.float32
_BF16 = jnp.bfloat16
_U32 = jnp.uint32


def _bits(x):
    return pltpu.bitcast(x, jnp.int32)


def _flt(x):
    return pltpu.bitcast(x, _F32)


def _ln(x):
    m = jnp.mean(x, axis=-1, keepdims=True)
    xc = x - m
    v = jnp.mean(xc * xc, axis=-1, keepdims=True)
    return xc * lax.rsqrt(v + EPS)


def _gelu(x):
    c = math.sqrt(2.0 / math.pi)
    inner = x * (c + (c * 0.044715) * (x * x))
    hx = 0.5 * x
    return hx + hx * jnp.tanh(inner)


def _dot(a, b):
    return jnp.dot(a, b, preferred_element_type=_F32)


def _dot_nt(a, b):
    return lax.dot_general(a, b, (((1,), (1,)), ((), ())), preferred_element_type=_F32)


def _dot_tn(a, b):
    return lax.dot_general(a, b, (((0,), (0,)), ((), ())), preferred_element_type=_F32)


def _kernel(x_hbm, wq_hbm, wk_hbm, wv_hbm, wo_hbm, win_hbm, wsp_hbm, bsp_hbm, wout_hbm,
            c_hbm, wmod_hbm, o_hbm,
            x_v, wq_v, h_v, b32_v, wo_v, win_v, wsp_v, bsp_v, wout_v, c_v, wmod_v,
            mod_v, wt_v, k_v, vt_v, kb_v, qf_v, nm_v, qs_v, l_v, ot_v, z_v,
            x1_v, z1_v, z2_v, out_v, sems, xsems, osems):
    def x_copy(r):
        rows = pl.ds(pl.multiple_of(r * RB, RB), RB)
        return pltpu.make_async_copy(x_hbm.at[0, rows], x_v.at[rows], xsems.at[r])

    early = {
        "c": pltpu.make_async_copy(c_hbm, c_v, sems.at[0]),
        "wq": pltpu.make_async_copy(wq_hbm, wq_v, sems.at[2]),
        "wk": pltpu.make_async_copy(wk_hbm, wt_v.at[pl.ds(0, DH)], sems.at[4]),
        "wv": pltpu.make_async_copy(wv_hbm, wt_v.at[pl.ds(DH, DH)], sems.at[3]),
        "wmod0": pltpu.make_async_copy(wmod_hbm.at[:, pl.ds(0, 2 * D)],
                                       wmod_v.at[:, pl.ds(0, 2 * D)], sems.at[1]),
    }
    late = {
        "wmod1": pltpu.make_async_copy(wmod_hbm.at[:, pl.ds(2 * D, 4 * D)],
                                       wmod_v.at[:, pl.ds(2 * D, 4 * D)], sems.at[6]),
        "wo": pltpu.make_async_copy(wo_hbm, wo_v, sems.at[7]),
        "win": pltpu.make_async_copy(win_hbm, win_v, sems.at[8]),
        "wsp": pltpu.make_async_copy(wsp_hbm, wsp_v, sems.at[9]),
        "bsp": pltpu.make_async_copy(bsp_hbm, bsp_v, sems.at[10]),
        "wout": pltpu.make_async_copy(wout_hbm, wout_v, sems.at[11]),
    }
    for cp in early.values():
        cp.start()
    x_copy(0).start()

    z_v[...] = jnp.zeros(z_v.shape, z_v.dtype)
    early["c"].wait()
    for r in range(1, NRB):
        x_copy(r).start()
    cf = c_v[...].astype(_F32)
    sc = (cf * jax.nn.sigmoid(cf)).astype(_BF16)
    sc8 = jnp.broadcast_to(sc, (16, D))

    with jax.named_scope("pre"):
        early["wq"].wait()
        wt_v[pl.ds(2 * DH, D), :] = wq_v[...].astype(_F32).T.astype(_BF16)
        x_copy(0).wait()
        xn0 = _ln(x_v[pl.ds(0, RB), :].astype(_F32))

        early["wmod0"].wait()
        mod_v[:, pl.ds(0, 2 * D)] = _dot(sc8, wmod_v[:, pl.ds(0, 2 * D)])[0:8]

        def modulate(xn):
            sa = mod_v[0:1, pl.ds(0, D)]
            ca = mod_v[0:1, pl.ds(D, D)]
            return (xn * (1.0 + ca) + sa).astype(_BF16)

        h_v[0] = modulate(xn0)
        early["wv"].wait()
        early["wk"].wait()

    def qkv_block(r, slot, kmax2):
        rows = pl.ds(pl.multiple_of(r * RB, RB), RB)
        rn = jnp.minimum(r + 1, NRB - 1)

        @pl.when(r + 1 < NRB)
        def _():
            x_copy(rn).wait()

        sub = lax.broadcasted_iota(jnp.int32, (128 - DH, RB), 0)
        one_row = jnp.where(sub == 0, 1.0, 0.0)
        t = _dot_nt(wt_v[...], h_v[slot])
        kt = t[0:DH].astype(_BF16).astype(_F32)
        kmax2 = jnp.maximum(kmax2, jnp.sum(kt * kt, axis=0, keepdims=True))
        kx = jnp.concatenate([kt, one_row], axis=0).T
        k_v[pl.ds(pl.multiple_of(r * (RB // 2), RB // 2), RB // 2), :] = pltpu.bitcast(
            kx[:, 0:2 * DH].astype(_BF16), _U32)
        for cc in range(RB // KC):
            kk = kx[cc * KC:cc * KC + 16]
            for d in range(DH):
                kb_v[r * (RB // KC) + cc, d] = jnp.broadcast_to(kk[:, d:d + 1], (16, 128))
        vt_v[:, rows] = pltpu.bitcast(t[DH:2 * DH].astype(_BF16), _U32)
        q = (t[2 * DH:] * QSCALE).astype(_BF16).astype(_F32).reshape(H, DH, RB)
        qf_v[:, :, rows] = q
        nm_v[:, rows] = jnp.sqrt(jnp.sum(q * q, axis=1))
        xn = _ln(x_v[pl.ds(pl.multiple_of(rn * RB, RB), RB), :].astype(_F32))
        h_v[1 - slot] = modulate(xn)
        return kmax2

    def qkv_body(j, kmax2):
        return qkv_block(2 * j + 1, 1, qkv_block(2 * j, 0, kmax2))

    with jax.named_scope("qkv"):
        kmax2 = lax.fori_loop(0, NRB // 2, qkv_body, jnp.zeros((1, RB), _F32))

    for cp in late.values():
        cp.start()

    kmax = jnp.sqrt(jnp.max(kmax2, axis=1, keepdims=True)) * (-1.01)
    nm_v[...] = (nm_v[...] * kmax).astype(_BF16).astype(_F32)

    def stage_idx(idx):
        qb = lax.shift_right_logical(idx, 5)
        h = lax.bitwise_and(idx, H - 1)
        return h, pl.ds(pl.multiple_of(qb * TQ, TQ), TQ)

    T = U * NKC
    stream = [(t, b) for t in range(T) for b in range(7, 0, -1)]
    NS = len(stream)
    cuts = {}
    for t in range(T):
        cuts.setdefault(min(7 * (t + 2) + DELTA, NS), []).append(t)
    gates, inserts = {}, {}
    for t in range(T):
        u = t // NKC
        for jj in range(NL):
            g = 7 * t + GOFF[jj]
            ins = min(max(g - LLAG, 7 * NKC * u - 1), 7 * NKC * (u + 1) - 1)
            inserts.setdefault(ins, []).append((t, jj))
            if g < NS:
                gates[g] = (t, jj)

    def att_body(j, carry):
        never = z_v[...] != 0
        st = {}
        for u in range(U):
            h, c = stage_idx(U * j + u)
            st[u] = dict(o=None, l=[None] * NL, h=h, c=c, qt=None)
        tiles = {t: [None] * 8 for t in range(T)}
        vp, gval = {}, {}

        def stage_setup(u):
            s_ = st[u]
            if s_["qt"] is not None:
                return
            q = qf_v[s_["h"], :, s_["c"]]
            nm = jnp.broadcast_to(nm_v[pl.ds(s_["h"], 1), s_["c"]], (DH, TQ))
            s_["qt"] = jnp.concatenate([q.astype(_BF16), nm.astype(_BF16)], axis=0)
            qs_v[u, 0:DH] = q
            qs_v[u, DH:DH + 8] = nm[0:8]

        def ladd(u, jj, x):
            l = st[u]["l"]
            l[jj] = x if l[jj] is None else l[jj] + x

        def vpu_unit(t, jj):
            u, kc = divmod(t, NKC)
            stage_setup(u)
            ls = pl.ds(128 * jj, 128)
            acc = [qs_v[u, DH:DH + 8, ls]] * 2
            for d in range(DH):
                qd = jnp.broadcast_to(qs_v[u, pl.ds(d, 1), ls], (8, 128))
                for a in range(2):
                    acc[a] = acc[a] + kb_v[kc, d, pl.ds(8 * a, 8), :] * qd
            p = [jnp.exp2(x) for x in acc]
            vp[(t, jj)] = jnp.concatenate(p, axis=0)
            ladd(u, jj, p[0] + p[1])
            gval[(t, jj)] = st[u]["l"][jj]

        def pv(t):
            u, kc = divmod(t, NKC)
            vt = pltpu.bitcast(vt_v[:, pl.ds(kc * KC, KC)], _BF16)
            tiles[t][0] = jnp.concatenate([vp[(t, jj)] for jj in range(NL)], axis=1)
            pb = jnp.concatenate(tiles[t], axis=0).astype(_BF16)
            o = _dot(vt, pb)
            s_ = st[u]
            s_["o"] = o if s_["o"] is None else o + s_["o"]
            if kc == NKC - 1:
                l = jnp.sum(jnp.concatenate(s_["l"], axis=1), axis=0, keepdims=True)
                ot_v[s_["h"], :, s_["c"]] = s_["o"] * (1.0 / l)
                l_v[pl.ds(s_["h"], 1), s_["c"]] = l

        def flush(group):
            if not group:
                return
            u = group[0][1] // NKC
            stage_setup(u)
            kb = []
            for i_, t, b in group:
                k_ = k_v[pl.ds((t % NKC) * (KC // 2) + 8 * b, 8), :]
                if i_ in gates:
                    pu = pltpu.bitcast(gval[gates[i_]], _U32)
                    k_ = jnp.where(never, pu[:, 0:2 * DH], k_)
                kb.append(k_)
            kk = pltpu.bitcast(jnp.concatenate(kb, axis=0), _BF16)
            s = _dot(kk, st[u]["qt"])
            for g_, (i_, t, b) in enumerate(group):
                p = jnp.exp2(s[16 * g_:16 * g_ + 16])
                a = p[0:8] + p[8:16]
                for jj in range(NL):
                    ladd(u, jj, a[:, 128 * jj:128 * jj + 128])
                tiles[t][b] = p
                for key in inserts.get(i_, []):
                    vpu_unit(*key)

        for key in inserts.get(-1, []):
            vpu_unit(*key)
        group = []
        for i_, (t, b) in enumerate(stream):
            if i_ in cuts or i_ % (7 * NKC) == 0 or len(group) >= LLAG:
                flush(group)
                group = []
            for tt in cuts.get(i_, []):
                pv(tt)
            group.append((i_, t, b))
        flush(group)
        for tt in cuts[NS]:
            pv(tt)
        return carry

    with jax.named_scope("att"):
        lax.fori_loop(0, NSTAGE // U, att_body, 0)

    lall = l_v[...]
    ok = jnp.logical_and(lall >= L_LO, lall <= L_HI)
    nbad = jnp.sum(jnp.where(ok, 0.0, 1.0))

    @pl.when(nbad > 0.0)
    def _():
        def slow_stage(idx, carry):
            h, c = stage_idx(idx)
            qt = jnp.concatenate([qf_v[h, :, c].astype(_BF16),
                                  jnp.zeros((DH, TQ), _BF16)], axis=0)

            def scores(kc):
                kr = pl.ds(pl.multiple_of(kc * (KC // 2), KC // 2), KC // 2)
                return _dot(pltpu.bitcast(k_v[kr, :], _BF16), qt)

            def max_body(kc, m):
                return jnp.maximum(m, jnp.max(scores(kc), axis=0, keepdims=True))

            m = lax.fori_loop(0, NKC, max_body, jnp.full((1, TQ), -jnp.inf, _F32))

            def pv_body(kc, lo):
                l, o = lo
                p = jnp.exp2(scores(kc) - m)
                ks = pl.ds(pl.multiple_of(kc * KC, KC), KC)
                vt = pltpu.bitcast(vt_v[:, ks], _BF16)
                return (l + jnp.sum(p, axis=0, keepdims=True),
                        o + _dot(vt, p.astype(_BF16)))

            l, o = lax.fori_loop(0, NKC, pv_body,
                                 (jnp.zeros((1, TQ), _F32), jnp.zeros((DH, TQ), _F32)))
            ot_v[h, :, c] = o * (1.0 / l)
            return carry

        lax.fori_loop(0, NSTAGE, slow_stage, 0)

    late["wmod1"].wait()
    mod_v[:, pl.ds(2 * D, 4 * D)] = _dot(sc8, wmod_v[:, pl.ds(2 * D, 4 * D)])[0:8]
    late["wo"].wait()
    late["win"].wait()

    def mid_block(rows):
        ga = mod_v[0:1, pl.ds(2 * D, D)]
        sb = mod_v[0:1, pl.ds(3 * D, D)]
        cb = mod_v[0:1, pl.ds(4 * D, D)]
        o = ot_v[:, :, rows].reshape(D, RB).T.astype(_BF16)
        a = _dot(o, wo_v[...])
        x1 = x_v[rows, :].astype(_F32) + ga * a
        x1_v[rows, :] = x1
        h2 = (_ln(x1) * (1.0 + cb) + sb).astype(_BF16)
        z1_v[rows, :] = _gelu(_dot(h2, win_v[:, pl.ds(0, FH)]))
        z2 = _gelu(_dot(h2, win_v[:, pl.ds(FH, FH)]))
        z2_v[rows, :] = _ln(z2).astype(_BF16)

    def mid_body(r, carry):
        for e in range(MU):
            mid_block(pl.ds(pl.multiple_of((r * MU + e) * RB, RB), RB))
        return carry

    if MU == NRB:
        for r in range(NRB):
            mid_block(pl.ds(r * RB, RB))
    else:
        with jax.named_scope("mid"):
            lax.fori_loop(0, NRB // MU, mid_body, 0)

    late["wsp"].wait()
    late["bsp"].wait()
    late["wout"].wait()
    b32_v[...] = bsp_v[...].astype(_F32)

    def out_copy(r):
        rows = pl.ds(pl.multiple_of(r * RB, RB), RB)
        return pltpu.make_async_copy(out_v.at[rows], o_hbm.at[0, rows], osems.at[r])

    def fin_block(r):
        rows = pl.ds(pl.multiple_of(r * RB, RB), RB)
        gb = mod_v[0:1, pl.ds(5 * D, D)]
        bcol = jnp.concatenate(
            [jnp.broadcast_to(b32_v[pl.ds(r * (RB // 128) + e, 1), :], (128, 128)).T
             for e in range(RB // 128)], axis=0)
        g = _dot(wsp_v[rows, :], z2_v[...])
        g = g + jnp.concatenate([bcol] * (FH // 128), axis=1)
        u = (z1_v[rows, :] * g).astype(_BF16)
        y = _dot(u, wout_v[...])
        out_v[rows, :] = (x1_v[rows, :] + gb * y).astype(_BF16)

    def fin_body(r, carry):
        for e in range(FU):
            fin_block(r * FU + e)
        for e in range(FU):
            out_copy(r * FU + e).start()
        return carry

    with jax.named_scope("fin"):
        lax.fori_loop(0, NRB // FU, fin_body, 0)
    for r in range(NRB):
        out_copy(r).wait()


@jax.jit
def pallas_adaLN_cond__grouped_kv_mqa__mixer_gmlp__prompt_kernel(
    A_x: jax.Array,
    A_wq: jax.Array,
    A_wk: jax.Array,
    A_wv: jax.Array,
    A_wo: jax.Array,
    B_x: jax.Array,
    B_w_in: jax.Array,
    B_w_sp: jax.Array,
    B_b_sp: jax.Array,
    B_w_out: jax.Array,
    c: jax.Array,
    w_mod: jax.Array,
):
    del B_x
    any_spec = pl.BlockSpec(memory_space=pl.ANY)
    scratch = [
        pltpu.VMEM((S, D), _BF16),
        pltpu.VMEM((D, D), _BF16),
        pltpu.VMEM((2, RB, D), _BF16),
        pltpu.VMEM((S // 128, 128), _F32),
        pltpu.VMEM((D, D), _BF16),
        pltpu.VMEM((D, F), _BF16),
        pltpu.VMEM((S, S), _BF16),
        pltpu.VMEM((S // 128, 128), _BF16),
        pltpu.VMEM((FH, D), _BF16),
        pltpu.VMEM((1, D), _BF16),
        pltpu.VMEM((D, 6 * D), _BF16),
        pltpu.VMEM((8, 6 * D), _F32),
        pltpu.VMEM((D + 2 * DH, D), _BF16),
        pltpu.VMEM((S // 2, 2 * DH), _U32),
        pltpu.VMEM((DH // 2, S), _U32),
        pltpu.VMEM((NKC, DH, 16, 128), _F32),
        pltpu.VMEM((H, DH, S), _F32),
        pltpu.VMEM((H, S), _F32),
        pltpu.VMEM((U, DH + 8, TQ), _F32),
        pltpu.VMEM((H, S), _F32),
        pltpu.VMEM((H, DH, S), _F32),
        pltpu.VMEM((8, 2 * DH), jnp.int32),
        pltpu.VMEM((S, D), _F32),
        pltpu.VMEM((S, FH), _F32),
        pltpu.VMEM((S, FH), _BF16),
        pltpu.VMEM((S, D), _BF16),
        pltpu.SemaphoreType.DMA((12,)),
        pltpu.SemaphoreType.DMA((NRB,)),
        pltpu.SemaphoreType.DMA((NRB,)),
    ]
    return pl.pallas_call(
        _kernel,
        out_shape=jax.ShapeDtypeStruct((1, S, D), _BF16),
        in_specs=[any_spec] * 11,
        out_specs=any_spec,
        scratch_shapes=scratch,
        compiler_params=pltpu.CompilerParams(vmem_limit_bytes=100 * 1024 * 1024),
        name="adaln_mqa_gmlp",
    )(A_x, A_wq, A_wk.T, A_wv.T, A_wo, B_w_in, B_w_sp, B_b_sp.reshape(S // 128, 128),
      B_w_out, c, w_mod)
```

```python
import math

import jax
import jax.numpy as jnp
from jax import lax
import jax.experimental.pallas as pl
import jax.experimental.pallas.tpu as pltpu

S = 2048
D = 512
H = 32
DH = 16
F = 1792
FH = F // 2
EPS = 1e-5

TQ = 512
KC = 128
NKC = S // KC
NQ = S // TQ
NSTAGE = NQ * H
NL = TQ // 128
U = 16
DELTA = 1
LLAG = 10
GOFF = (8, 10, 12, 14)
L_LO = 2.0 ** -40
L_HI = 2.0 * S

RB = 256
NRB = S // RB
MU = 2
ZSTEP = 5
OB = 256
FU = 1

QSCALE = (DH ** -0.5) * math.log2(math.e)

_F32 = jnp.float32
_BF16 = jnp.bfloat16
_U32 = jnp.uint32


def _bits(x):
    return pltpu.bitcast(x, jnp.int32)


def _flt(x):
    return pltpu.bitcast(x, _F32)


def _ln(x):
    m = jnp.mean(x, axis=-1, keepdims=True)
    xc = x - m
    v = jnp.mean(xc * xc, axis=-1, keepdims=True)
    return xc * lax.rsqrt(v + EPS)


def _gelu(x):
    c = math.sqrt(2.0 / math.pi)
    inner = x * (c + (c * 0.044715) * (x * x))
    hx = 0.5 * x
    return hx + hx * jnp.tanh(inner)


def _fold8(x):
    n, _, lanes = x.shape
    sub = lax.broadcasted_iota(jnp.int32, (8, lanes), 0)
    m4, m2, m1 = sub < 4, (sub & 2) == 0, (sub & 1) == 0
    out = []
    for g in range(n // 8):
        v = [x[8 * g + i] for i in range(8)]
        c = [jnp.where(m4, v[i], v[i + 4])
             + pltpu.roll(jnp.where(m4, v[i + 4], v[i]), 4, 0) for i in range(4)]
        d = [jnp.where(m2, c[i] + pltpu.roll(c[i], 6, 0),
                       c[i + 2] + pltpu.roll(c[i + 2], 2, 0)) for i in range(2)]
        out.append(jnp.where(m1, d[0] + pltpu.roll(d[0], 7, 0),
                             d[1] + pltpu.roll(d[1], 1, 0)))
    return jnp.concatenate(out, axis=0)


def _dot(a, b):
    return jnp.dot(a, b, preferred_element_type=_F32)


def _dot_nt(a, b):
    return lax.dot_general(a, b, (((1,), (1,)), ((), ())), preferred_element_type=_F32)


def _dot_tn(a, b):
    return lax.dot_general(a, b, (((0,), (0,)), ((), ())), preferred_element_type=_F32)


def _kernel(x_hbm, wq_hbm, wk_hbm, wv_hbm, wo_hbm, win_hbm, wsp_hbm, bsp_hbm, wout_hbm,
            c_hbm, wmod_hbm, o_hbm,
            x_v, wq_v, h_v, b32_v, wo_v, win_v, wsp_v, bsp_v, wout_v, c_v, wmod_v,
            mod_v, wt_v, k_v, vt_v, kb_v, qf_v, nm_v, qs_v, l_v, ot_v, z_v,
            x1_v, z1_v, z2_v, zf_v, on_v, inv_v, out_v, zm_v, zs_s, sems):
    def x_copy(i):
        if isinstance(i, int) and i in (0, NRB // 2):
            rows = pl.ds(max(2 * i - 1, 0) * RB, RB)
        else:
            rows = pl.ds(pl.multiple_of((2 * i - 1) * RB, RB), 2 * RB)
        return pltpu.make_async_copy(x_hbm.at[0, rows], x_v.at[rows], sems.at[4 + i])

    early = {
        "c": pltpu.make_async_copy(c_hbm, c_v, sems.at[0]),
        "wq": pltpu.make_async_copy(wq_hbm, wq_v, sems.at[1]),
        "wk": pltpu.make_async_copy(wk_hbm, wt_v.at[pl.ds(0, DH)], sems.at[2]),
        "wv": pltpu.make_async_copy(wv_hbm, wt_v.at[pl.ds(DH, DH)], sems.at[2]),
        "wmod0": pltpu.make_async_copy(wmod_hbm.at[:, pl.ds(0, 2 * D)],
                                       wmod_v.at[:, pl.ds(0, 2 * D)], sems.at[3]),
    }
    late = {
        "wmod1": pltpu.make_async_copy(wmod_hbm.at[:, pl.ds(2 * D, 4 * D)],
                                       wmod_v.at[:, pl.ds(2 * D, 4 * D)], sems.at[0]),
        "wo": pltpu.make_async_copy(wo_hbm, wo_v, sems.at[0]),
        "win": pltpu.make_async_copy(win_hbm, win_v, sems.at[0]),
        "wsp": pltpu.make_async_copy(wsp_hbm, wsp_v, sems.at[1]),
        "bsp": pltpu.make_async_copy(bsp_hbm, bsp_v, sems.at[1]),
        "wout": pltpu.make_async_copy(wout_hbm, wout_v, sems.at[1]),
    }
    early["c"].start()
    early["wq"].start()
    x_copy(0).start()
    early["wk"].start()
    early["wv"].start()
    early["wmod0"].start()

    z_v[...] = jnp.zeros(z_v.shape, z_v.dtype)
    zm_v[...] = jnp.zeros(zm_v.shape, zm_v.dtype)
    zs_s[0] = 0
    early["c"].wait()
    cf = c_v[...].astype(_F32)
    sc = (cf * jax.nn.sigmoid(cf)).astype(_BF16)
    sc8 = jnp.broadcast_to(sc, (16, D))

    early["wq"].wait()
    for i in range(1, NRB // 2 + 1):
        x_copy(i).start()
    wt_v[pl.ds(2 * DH, D), :] = wq_v[...].astype(_F32).T.astype(_BF16)
    x_copy(0).wait()
    xn0 = _ln(x_v[pl.ds(0, RB), :].astype(_F32))

    early["wmod0"].wait()
    mod_v[:, pl.ds(0, 2 * D)] = _dot(sc8, wmod_v[:, pl.ds(0, 2 * D)])[0:8]

    def modulate(xn):
        sa = mod_v[0:1, pl.ds(0, D)]
        ca = mod_v[0:1, pl.ds(D, D)]
        return (xn * (1.0 + ca) + sa).astype(_BF16)

    h_v[0] = modulate(xn0)
    early["wv"].wait()
    early["wk"].wait()

    def qkv_block(r, slot, kmax2):
        rows = pl.ds(pl.multiple_of(r * RB, RB), RB)
        rn = jnp.minimum(r + 1, NRB - 1)

        sub = lax.broadcasted_iota(jnp.int32, (128 - DH, RB), 0)
        one_row = jnp.where(sub == 1, 1.0, 0.0)
        t = _dot_nt(wt_v[...], h_v[slot])
        kt = t[0:DH].astype(_BF16).astype(_F32)
        kmax2 = jnp.maximum(kmax2, jnp.sum(kt * kt, axis=0, keepdims=True))
        kx = jnp.concatenate([kt, one_row], axis=0).T
        k_v[pl.ds(pl.multiple_of(r * (RB // 2), RB // 2), RB // 2), :] = pltpu.bitcast(
            kx[:, 0:2 * DH].astype(_BF16), _U32)
        for cc in range(RB // KC):
            kk = kx[cc * KC:cc * KC + 16]
            for d in range(DH):
                kb_v[r * (RB // KC) + cc, d] = jnp.broadcast_to(kk[:, d:d + 1], (16, 128))
        vt_v[:, rows] = pltpu.bitcast(t[DH:2 * DH].astype(_BF16), _U32)
        q = (t[2 * DH:] * QSCALE).astype(_BF16).astype(_F32).reshape(H, DH, RB)
        qf_v[:, :, rows] = q
        q2 = q * q
        nm_v[:, rows] = jnp.sqrt(_fold8(q2[:, 0:8] + q2[:, 8:16]))
        xn = _ln(x_v[pl.ds(pl.multiple_of(rn * RB, RB), RB), :].astype(_F32))
        h_v[1 - slot] = modulate(xn)
        return kmax2

    def qkv_body(j, kmax2):
        @pl.when(j + 1 < NRB // 2)
        def _():
            x_copy(jnp.minimum(j + 1, NRB // 2 - 1)).wait()

        @pl.when(j + 1 == NRB // 2)
        def _():
            x_copy(NRB // 2).wait()

        return qkv_block(2 * j + 1, 1, qkv_block(2 * j, 0, kmax2))

    kmax2 = lax.fori_loop(0, NRB // 2, qkv_body, jnp.zeros((1, RB), _F32))

    for cp in late.values():
        cp.start()

    kmax = jnp.sqrt(jnp.max(kmax2, axis=1, keepdims=True)) * (-1.01)
    nm_v[...] = (nm_v[...] * kmax).astype(_BF16).astype(_F32)

    def stage_idx(idx):
        qb = lax.shift_right_logical(idx, 5)
        h = lax.bitwise_and(idx, H - 1)
        return h, pl.ds(pl.multiple_of(qb * TQ, TQ), TQ)

    T = U * NKC
    stream = [(t, b) for t in range(T) for b in range(7, 0, -1)]
    NS = len(stream)
    cuts = {}
    for t in range(T):
        cuts.setdefault(min(7 * (t + 2) + DELTA, NS), []).append(t)
    gates, inserts = {}, {}
    for t in range(T):
        u = t // NKC
        for jj in range(NL):
            g = 7 * t + GOFF[jj]
            ins = min(max(g - LLAG, 7 * NKC * u - 1), 7 * NKC * (u + 1) - 1)
            inserts.setdefault(ins, []).append((t, jj))
            if g < NS:
                gates[g] = (t, jj)

    def att_body(j, carry):
        never = z_v[...] != 0
        st = {}
        for u in range(U):
            h, c = stage_idx(U * j + u)
            st[u] = dict(o=None, l=[None] * NL, h=h, c=c, qt=None)
        tiles = {t: [None] * 8 for t in range(T)}
        vp, gval = {}, {}
        lim = list(carry)

        def stage_setup(u):
            s_ = st[u]
            if s_["qt"] is not None:
                return
            q = qf_v[s_["h"], :, s_["c"]]
            nm = jnp.broadcast_to(nm_v[pl.ds(s_["h"], 1), s_["c"]], (8, TQ))
            s_["qt"] = jnp.concatenate([q.astype(_BF16), pltpu.bitcast(nm, _BF16)], axis=0)
            qs_v[u, 0:DH] = q
            qs_v[u, DH:DH + 8] = nm

        def ladd(u, jj, x):
            l = st[u]["l"]
            l[jj] = x if l[jj] is None else l[jj] + x

        def vpu_unit(t, jj):
            u, kc = divmod(t, NKC)
            stage_setup(u)
            ls = pl.ds(128 * jj, 128)
            acc = [qs_v[u, DH:DH + 8, ls]] * 2
            for d in range(DH):
                qd = jnp.broadcast_to(qs_v[u, pl.ds(d, 1), ls], (8, 128))
                for a in range(2):
                    acc[a] = acc[a] + kb_v[kc, d, pl.ds(8 * a, 8), :] * qd
            p = [jnp.exp2(x) for x in acc]
            vp[(t, jj)] = jnp.concatenate(p, axis=0)
            ladd(u, jj, p[0] + p[1])
            gval[(t, jj)] = st[u]["l"][jj]

        def pv(t):
            u, kc = divmod(t, NKC)
            vt = pltpu.bitcast(vt_v[:, pl.ds(kc * KC, KC)], _BF16)
            tiles[t][0] = jnp.concatenate([vp[(t, jj)] for jj in range(NL)], axis=1)
            pb = jnp.concatenate(tiles[t], axis=0).astype(_BF16)
            o = _dot(vt, pb)
            s_ = st[u]
            s_["o"] = o if s_["o"] is None else o + s_["o"]
            if kc == NKC - 1:
                ot_v[s_["h"], :, s_["c"]] = s_["o"]
                l_v[s_["h"], :, s_["c"]] = jnp.concatenate(s_["l"], axis=1)
                for x in s_["l"]:
                    lim[0] = jnp.minimum(lim[0], x)
                    lim[1] = jnp.maximum(lim[1], x)

        def flush(group):
            if not group:
                return
            u = group[0][1] // NKC
            stage_setup(u)
            kb = []
            for i_, t, b in group:
                k_ = k_v[pl.ds((t % NKC) * (KC // 2) + 8 * b, 8), :]
                if i_ in gates:
                    pu = pltpu.bitcast(gval[gates[i_]], _U32)
                    k_ = jnp.where(never, pu[:, 0:2 * DH], k_)
                kb.append(k_)
            kk = pltpu.bitcast(jnp.concatenate(kb, axis=0), _BF16)
            s = _dot(kk, st[u]["qt"])
            for g_, (i_, t, b) in enumerate(group):
                p = jnp.exp2(s[16 * g_:16 * g_ + 16])
                a = p[0:8] + p[8:16]
                for jj in range(NL):
                    ladd(u, jj, a[:, 128 * jj:128 * jj + 128])
                tiles[t][b] = p
                for key in inserts.get(i_, []):
                    vpu_unit(*key)

        for key in inserts.get(-1, []):
            vpu_unit(*key)
        group = []
        for i_, (t, b) in enumerate(stream):
            if i_ in cuts or i_ % (7 * NKC) == 0 or len(group) >= LLAG:
                flush(group)
                group = []
            for tt in cuts.get(i_, []):
                pv(tt)
            group.append((i_, t, b))
        flush(group)
        for tt in cuts[NS]:
            pv(tt)
        return tuple(lim)

    lmin, lmax = lax.fori_loop(0, NSTAGE // U, att_body,
                               (jnp.ones((8, 128), _F32), jnp.ones((8, 128), _F32)))

    ok = jnp.logical_and(lmin >= L_LO, lmax <= L_HI)
    nbad = jnp.sum(jnp.where(ok, 0.0, 1.0))

    @pl.when(nbad > 0.0)
    def _():
        def slow_stage(idx, carry):
            h, c = stage_idx(idx)
            qt = jnp.concatenate([qf_v[h, :, c].astype(_BF16),
                                  jnp.zeros((DH, TQ), _BF16)], axis=0)

            def scores(kc):
                kr = pl.ds(pl.multiple_of(kc * (KC // 2), KC // 2), KC // 2)
                return _dot(pltpu.bitcast(k_v[kr, :], _BF16), qt)

            def max_body(kc, m):
                return jnp.maximum(m, jnp.max(scores(kc), axis=0, keepdims=True))

            m = lax.fori_loop(0, NKC, max_body, jnp.full((1, TQ), -jnp.inf, _F32))

            def pv_body(kc, lo):
                l, o = lo
                p = jnp.exp2(scores(kc) - m)
                ks = pl.ds(pl.multiple_of(kc * KC, KC), KC)
                vt = pltpu.bitcast(vt_v[:, ks], _BF16)
                return (l + jnp.sum(p.reshape(KC // 8, 8, TQ), axis=0),
                        o + _dot(vt, p.astype(_BF16)))

            l, o = lax.fori_loop(0, NKC, pv_body,
                                 (jnp.zeros((8, TQ), _F32), jnp.zeros((DH, TQ), _F32)))
            ot_v[h, :, c] = o
            l_v[h, :, c] = l
            return carry

        lax.fori_loop(0, NSTAGE, slow_stage, 0)

    def attn_rows(r, e):
        rows = pl.ds(pl.multiple_of(r * RB, RB), RB)
        inv_v[e] = 1.0 / _fold8(l_v[:, :, rows])
        o = jnp.concatenate(
            [ot_v[h, :, rows] * jnp.broadcast_to(inv_v[e, pl.ds(h, 1), :], (DH, RB))
             for h in range(H)], axis=0)
        return o.T.astype(_BF16)

    late["wmod1"].wait()
    late["wo"].wait()
    late["win"].wait()
    mod_v[:, pl.ds(2 * D, 4 * D)] = _dot(sc8, wmod_v[:, pl.ds(2 * D, 4 * D)])[0:8]
    on_v[...] = pltpu.bitcast(attn_rows(0, 0), _U32)

    def mid_a(rows, o):
        ga = mod_v[0:1, pl.ds(2 * D, D)]
        sb = mod_v[0:1, pl.ds(3 * D, D)]
        cb = mod_v[0:1, pl.ds(4 * D, D)]
        a = _dot(o, wo_v[...])
        x1 = x_v[rows, :].astype(_F32) + ga * a
        x1_v[rows, :] = x1
        return (_ln(x1) * (1.0 + cb) + sb).astype(_BF16)

    def paced_ln(x, pace, step):
        never = zm_v[...] != 0
        n = x.shape[1]
        rg = pace.shape[0] // 16
        out = []
        for g in range(x.shape[0] // 16):
            xg = x[16 * g:16 * g + 16]
            s = xg[:, 0:128]
            for j in range(1, n // 128):
                s = s + xg[:, 128 * j:128 * j + 128]
            j, i = divmod(step * g, rg)
            s = jnp.where(never, pace[16 * i:16 * i + 16, 128 * j:128 * j + 128], s)
            xc = xg - jnp.sum(s, axis=1, keepdims=True) * (1.0 / n)
            v = jnp.mean(xc * xc, axis=1, keepdims=True)
            out.append(xc * lax.rsqrt(v + EPS))
        return jnp.concatenate(out, axis=0)

    def mid_b(rows, h2, e):
        zf_v[e] = _gelu(_dot(h2, win_v[:, pl.ds(FH, FH)]))
        z1 = _gelu(_dot(h2, win_v[:, pl.ds(0, FH)]))
        z1_v[rows, :] = z1
        z2_v[rows, :] = paced_ln(zf_v[e + zs_s[0]], z1, ZSTEP).astype(_BF16)

    def mid_body(r, carry):
        rows = [pl.ds(pl.multiple_of((r * MU + e) * RB, RB), RB) for e in range(MU)]
        os_ = [pltpu.bitcast(on_v[...], _BF16)] + [attn_rows(r * MU + e, e) for e in range(1, MU)]
        h2 = [mid_a(rw, o) for rw, o in zip(rows, os_)]
        for e, (rw, h) in enumerate(zip(rows, h2)):
            if e == MU - 1:
                on_v[...] = pltpu.bitcast(attn_rows(jnp.minimum((r + 1) * MU, NRB - 1), 0), _U32)
            mid_b(rw, h, e)
        return carry

    lax.fori_loop(0, NRB // MU, mid_body, 0)

    late["wsp"].wait()
    late["bsp"].wait()
    late["wout"].wait()
    b32_v[...] = bsp_v[...].astype(_F32)

    def out_copy(i):
        rows = pl.ds(pl.multiple_of(i * OB, OB), OB)
        return pltpu.make_async_copy(out_v.at[rows], o_hbm.at[0, rows], sems.at[2])

    def fin_block(r):
        rows = pl.ds(pl.multiple_of(r * RB, RB), RB)
        gb = mod_v[0:1, pl.ds(5 * D, D)]
        bcol = jnp.concatenate(
            [jnp.broadcast_to(b32_v[pl.ds(r * (RB // 128) + e, 1), :], (128, 128)).T
             for e in range(RB // 128)], axis=0)
        g = _dot(wsp_v[rows, :], z2_v[...])
        g = g + jnp.concatenate([bcol] * (FH // 128), axis=1)
        u = (z1_v[rows, :] * g).astype(_BF16)
        y = _dot(u, wout_v[...])
        out_v[rows, :] = (x1_v[rows, :] + gb * y).astype(_BF16)

    def fin_body(r, carry):
        for e in range(FU):
            fin_block(r * FU + e)
        for e in range(FU * RB // OB):
            out_copy(r * (FU * RB // OB) + e).start()
        return carry

    lax.fori_loop(0, NRB // FU, fin_body, 0)
    for i in range(S // OB):
        out_copy(i).wait()


@jax.jit
def pallas_adaLN_cond__grouped_kv_mqa__mixer_gmlp__prompt_kernel(
    A_x: jax.Array,
    A_wq: jax.Array,
    A_wk: jax.Array,
    A_wv: jax.Array,
    A_wo: jax.Array,
    B_x: jax.Array,
    B_w_in: jax.Array,
    B_w_sp: jax.Array,
    B_b_sp: jax.Array,
    B_w_out: jax.Array,
    c: jax.Array,
    w_mod: jax.Array,
):
    del B_x
    any_spec = pl.BlockSpec(memory_space=pl.ANY)
    scratch = [
        pltpu.VMEM((S, D), _BF16),
        pltpu.VMEM((D, D), _BF16),
        pltpu.VMEM((2, RB, D), _BF16),
        pltpu.VMEM((S // 128, 128), _F32),
        pltpu.VMEM((D, D), _BF16),
        pltpu.VMEM((D, F), _BF16),
        pltpu.VMEM((S, S), _BF16),
        pltpu.VMEM((S // 128, 128), _BF16),
        pltpu.VMEM((FH, D), _BF16),
        pltpu.VMEM((1, D), _BF16),
        pltpu.VMEM((D, 6 * D), _BF16),
        pltpu.VMEM((8, 6 * D), _F32),
        pltpu.VMEM((D + 2 * DH, D), _BF16),
        pltpu.VMEM((S // 2, 2 * DH), _U32),
        pltpu.VMEM((DH // 2, S), _U32),
        pltpu.VMEM((NKC, DH, 16, 128), _F32),
        pltpu.VMEM((H, DH, S), _F32),
        pltpu.VMEM((H, S), _F32),
        pltpu.VMEM((U, DH + 8, TQ), _F32),
        pltpu.VMEM((H, 8, S), _F32),
        pltpu.VMEM((H, DH, S), _F32),
        pltpu.VMEM((8, 2 * DH), jnp.int32),
        pltpu.VMEM((S, D), _F32),
        pltpu.VMEM((S, FH), _F32),
        pltpu.VMEM((S, FH), _BF16),
        pltpu.VMEM((MU, RB, FH), _F32),
        pltpu.VMEM((RB // 2, D), _U32),
        pltpu.VMEM((MU, H, RB), _F32),
        pltpu.VMEM((S, D), _BF16),
        pltpu.VMEM((16, 128), jnp.int32),
        pltpu.SMEM((1,), jnp.int32),
        pltpu.SemaphoreType.DMA((5 + NRB // 2,)),
    ]
    return pl.pallas_call(
        _kernel,
        out_shape=jax.ShapeDtypeStruct((1, S, D), _BF16),
        in_specs=[any_spec] * 11,
        out_specs=any_spec,
        scratch_shapes=scratch,
        compiler_params=pltpu.CompilerParams(vmem_limit_bytes=100 * 1024 * 1024),
        name="adaln_mqa_gmlp",
    )(A_x, A_wq, A_wk.T, A_wv.T, A_wo, B_w_in, B_w_sp, B_b_sp.reshape(S // 128, 128),
      B_w_out, c, w_mod)
```

```python
import math

import jax
import jax.numpy as jnp
from jax import lax
import jax.experimental.pallas as pl
import jax.experimental.pallas.tpu as pltpu

S = 2048
D = 512
H = 32
DH = 16
F = 1792
FH = F // 2
EPS = 1e-5

TQ = 512
KC = 128
NKC = S // KC
NQ = S // TQ
NSTAGE = NQ * H
NL = TQ // 128
U = 16
DELTA = 1
DPOS = 4
LLAG = 10
GOFF = (8, 10, 12, 14)
L_LO = 2.0 ** -40
L_HI = 2.0 * S

RB = 256
NRB = S // RB
MU = 2
ZSTEP = 6
HSTEP = (2, 5)
OG = (-1, -1, -1, -1, -1, -1, -1, 3)
OSTEP = (4, 8)
QSTEP = (0, 2)
OB = (256, 64)

QSCALE = (DH ** -0.5) * math.log2(math.e)

_F32 = jnp.float32
_BF16 = jnp.bfloat16
_U32 = jnp.uint32


def _bits(x):
    return pltpu.bitcast(x, jnp.int32)


def _flt(x):
    return pltpu.bitcast(x, _F32)


def _ln(x):
    m = jnp.mean(x, axis=-1, keepdims=True)
    xc = x - m
    v = jnp.mean(xc * xc, axis=-1, keepdims=True)
    return xc * lax.rsqrt(v + EPS)


def _gelu(x):
    c = math.sqrt(2.0 / math.pi)
    inner = x * (c + (c * 0.044715) * (x * x))
    hx = 0.5 * x
    return hx + hx * jnp.tanh(inner)


def _fold8(x):
    n, _, lanes = x.shape
    sub = lax.broadcasted_iota(jnp.int32, (8, lanes), 0)
    m4, m2, m1 = sub < 4, (sub & 2) == 0, (sub & 1) == 0
    out = []
    for g in range(n // 8):
        v = [x[8 * g + i] for i in range(8)]
        c = [jnp.where(m4, v[i], v[i + 4])
             + pltpu.roll(jnp.where(m4, v[i + 4], v[i]), 4, 0) for i in range(4)]
        d = [jnp.where(m2, c[i] + pltpu.roll(c[i], 6, 0),
                       c[i + 2] + pltpu.roll(c[i + 2], 2, 0)) for i in range(2)]
        out.append(jnp.where(m1, d[0] + pltpu.roll(d[0], 7, 0),
                             d[1] + pltpu.roll(d[1], 1, 0)))
    return jnp.concatenate(out, axis=0)


def _dot(a, b):
    return jnp.dot(a, b, preferred_element_type=_F32)


def _dot_nt(a, b):
    return lax.dot_general(a, b, (((1,), (1,)), ((), ())), preferred_element_type=_F32)


def _dot_tn(a, b):
    return lax.dot_general(a, b, (((0,), (0,)), ((), ())), preferred_element_type=_F32)


def _kernel(x_hbm, wq_hbm, wk_hbm, wv_hbm, wo_hbm, win_hbm, wsp_hbm, bsp_hbm, wout_hbm,
            c_hbm, wmod_hbm, o_hbm,
            x_v, wq_v, h_v, b32_v, wo_v, win_v, wsp_v, bsp_v, wout_v, c_v, wmod_v,
            mod_v, wt_v, wkv_v, k_v, vt_v, kb_v, qf_v, nm_v, qs_v, l_v, ot_v, z_v,
            x1a_v, x1b_v, z1_v, z2_v, zfa_v, zfb_v, on_v, inv_v, out_v, zm_v, ps_v, po_v, zs_s, sems):
    x1_v, zf_v = (x1a_v, x1b_v), (zfa_v, zfb_v)

    def x_copy(i):
        if isinstance(i, int) and i in (0, NRB // 2):
            rows = pl.ds(max(2 * i - 1, 0) * RB, RB)
        else:
            rows = pl.ds(pl.multiple_of((2 * i - 1) * RB, RB), 2 * RB)
        return pltpu.make_async_copy(x_hbm.at[0, rows], x_v.at[rows], sems.at[4 + i])

    early = {
        "c": pltpu.make_async_copy(c_hbm, c_v, sems.at[0]),
        "wq": pltpu.make_async_copy(wq_hbm, wq_v, sems.at[1]),
        "wk": pltpu.make_async_copy(wk_hbm, wkv_v.at[pl.ds(0, DH)], sems.at[2]),
        "wv": pltpu.make_async_copy(wv_hbm, wkv_v.at[pl.ds(DH, DH)], sems.at[2]),
        "wmod0": pltpu.make_async_copy(wmod_hbm.at[:, pl.ds(0, 2 * D)],
                                       wmod_v.at[:, pl.ds(0, 2 * D)], sems.at[3]),
    }
    late = {
        "wmod1": pltpu.make_async_copy(wmod_hbm.at[:, pl.ds(2 * D, 4 * D)],
                                       wmod_v.at[:, pl.ds(2 * D, 4 * D)], sems.at[0]),
        "wo": pltpu.make_async_copy(wo_hbm, wo_v, sems.at[0]),
        "win": pltpu.make_async_copy(win_hbm, win_v, sems.at[0]),
        "wsp": pltpu.make_async_copy(wsp_hbm, wsp_v, sems.at[1]),
        "bsp": pltpu.make_async_copy(bsp_hbm, bsp_v, sems.at[1]),
        "wout": pltpu.make_async_copy(wout_hbm, wout_v, sems.at[1]),
    }
    early["c"].start()
    early["wq"].start()
    x_copy(0).start()
    early["wk"].start()
    early["wv"].start()
    early["wmod0"].start()

    z_v[...] = jnp.zeros(z_v.shape, z_v.dtype)
    zm_v[...] = jnp.zeros(zm_v.shape, zm_v.dtype)
    ps_v[...] = jnp.zeros(ps_v.shape, ps_v.dtype)
    po_v[...] = jnp.zeros(po_v.shape, po_v.dtype)
    zs_s[0] = 0
    early["c"].wait()
    cf = c_v[...].astype(_F32)
    sc = (cf * jax.nn.sigmoid(cf)).astype(_BF16)
    sc8 = jnp.broadcast_to(sc, (16, D))

    early["wq"].wait()
    for i in range(1, NRB // 2 + 1):
        x_copy(i).start()
    wt_v[pl.ds(DH, D // 2), :] = pltpu.bitcast(wq_v[...].astype(_F32).T.astype(_BF16), _U32)
    x_copy(0).wait()
    early["wv"].wait()
    early["wk"].wait()
    wt_v[pl.ds(0, DH), :] = pltpu.bitcast(wkv_v[...], _U32)
    xn0 = _ln(x_v[pl.ds(0, RB), :].astype(_F32))

    early["wmod0"].wait()
    mod_v[:, pl.ds(0, 2 * D)] = _dot(sc8, wmod_v[:, pl.ds(0, 2 * D)])[0:8]

    def modulate(xn):
        sa = mod_v[0:1, pl.ds(0, D)]
        ca = mod_v[0:1, pl.ds(D, D)]
        return pltpu.bitcast((xn * (1.0 + ca) + sa).astype(_BF16), _U32)

    h_v[0] = modulate(xn0)

    def paced_ln(x, pace, step):
        never = zm_v[...] != 0
        n = x.shape[1]
        rg = pace.shape[0] // 16
        out = []
        for g in range(x.shape[0] // 16):
            xg = x[16 * g:16 * g + 16]
            s = xg[:, 0:128]
            for j in range(1, n // 128):
                s = s + xg[:, 128 * j:128 * j + 128]
            j, i = divmod(step * g, rg)
            s = jnp.where(never, pace[16 * i:16 * i + 16, 128 * j:128 * j + 128], s)
            xc = xg - jnp.sum(s, axis=1, keepdims=True) * (1.0 / n)
            v = jnp.mean(xc * xc, axis=1, keepdims=True)
            out.append(xc * lax.rsqrt(v + EPS))
        return jnp.concatenate(out, axis=0)

    def qkv_block(r, slot, kmax2):
        rows = pl.ds(pl.multiple_of(r * RB, RB), RB)
        rn = jnp.minimum(r + 1, NRB - 1)

        sub = lax.broadcasted_iota(jnp.int32, (128 - DH, RB), 0)
        one_row = jnp.where(sub == 1, 1.0, 0.0)
        t = _dot_nt(pltpu.bitcast(wt_v[...], _BF16), pltpu.bitcast(h_v[slot], _BF16))
        kt = t[0:DH].astype(_BF16).astype(_F32)
        kmax2 = jnp.maximum(kmax2, jnp.sum(kt * kt, axis=0, keepdims=True))
        kx = jnp.concatenate([kt, one_row], axis=0).T
        k_v[pl.ds(pl.multiple_of(r * (RB // 2), RB // 2), RB // 2), :] = pltpu.bitcast(
            kx[:, 0:2 * DH].astype(_BF16), _U32)
        for cc in range(RB // KC):
            kk = kx[cc * KC:cc * KC + 16]
            for d in range(DH):
                kb_v[r * (RB // KC) + cc, d] = jnp.broadcast_to(kk[:, d:d + 1], (16, 128))
        vt_v[:, rows] = pltpu.bitcast(t[DH:2 * DH].astype(_BF16), _U32)
        q = (t[2 * DH:] * QSCALE).astype(_BF16).astype(_F32).reshape(H, DH, RB)
        qf_v[:, :, rows] = q
        q2 = q * q
        nm_v[:, rows] = jnp.sqrt(_fold8(q2[:, 0:8] + q2[:, 8:16]))
        xn = x_v[pl.ds(pl.multiple_of(rn * RB, RB), RB), :].astype(_F32)
        st_ = QSTEP[slot]
        xn = paced_ln(xn, t, st_) if st_ else _ln(xn)
        h_v[1 - slot] = modulate(xn)
        return kmax2

    def qkv_body(j, kmax2):
        @pl.when(j + 1 < NRB // 2)
        def _():
            x_copy(jnp.minimum(j + 1, NRB // 2 - 1)).wait()

        @pl.when(j + 1 == NRB // 2)
        def _():
            x_copy(NRB // 2).wait()

        return qkv_block(2 * j + 1, 1, qkv_block(2 * j, 0, kmax2))

    kmax2 = lax.fori_loop(0, NRB // 2, qkv_body, jnp.zeros((1, RB), _F32))

    for cp in late.values():
        cp.start()

    kmax = jnp.sqrt(jnp.max(kmax2, axis=1, keepdims=True)) * (-1.01)
    nm_v[...] = (nm_v[...] * kmax).astype(_BF16).astype(_F32)

    def stage_idx(idx):
        if isinstance(idx, int):
            return idx % H, pl.ds((idx // H) * TQ, TQ)
        qb = lax.shift_right_logical(idx, 5)
        h = lax.bitwise_and(idx, H - 1)
        return h, pl.ds(pl.multiple_of(qb * TQ, TQ), TQ)

    T = U * NKC
    stream = [(t, b) for t in range(T) for b in range(7, 0, -1)]
    NS = len(stream)
    cuts = {}
    for t in range(T):
        cuts.setdefault(min(7 * (t + 2) + DELTA, NS), []).append(t)
    gates, inserts = {}, {}
    for t in range(T):
        u = t // NKC
        for jj in range(NL):
            g = 7 * t + GOFF[jj]
            ins = min(max(g - LLAG, 7 * NKC * u - 1), 7 * NKC * (u + 1) - 1)
            inserts.setdefault(ins, []).append((t, jj))
            if g < NS:
                gates[g] = (t, jj)

    def pv_deferred(idx):
        h, c = stage_idx(idx)
        vt = pltpu.bitcast(vt_v[:, pl.ds(S - KC, KC)], _BF16)
        ot_v[h, :, c] = po_v[...] + _dot(vt, pltpu.bitcast(ps_v[...], _BF16))

    def att_body(j, carry):
        never = z_v[...] != 0
        st = {}
        for u in range(U):
            h, c = stage_idx(U * j + u)
            st[u] = dict(o=None, l=[None] * NL, h=h, c=c, qt=None)
        tiles = {t: [None] * 8 for t in range(T)}
        vp, gval = {}, {}
        lim = list(carry)

        def stage_setup(u):
            s_ = st[u]
            if s_["qt"] is not None:
                return
            q = qf_v[s_["h"], :, s_["c"]]
            nm = jnp.broadcast_to(nm_v[pl.ds(s_["h"], 1), s_["c"]], (8, TQ))
            s_["qt"] = jnp.concatenate([q.astype(_BF16), pltpu.bitcast(nm, _BF16)], axis=0)
            qs_v[u, 0:DH] = q
            qs_v[u, DH:DH + 8] = nm

        def ladd(u, jj, x):
            l = st[u]["l"]
            l[jj] = x if l[jj] is None else l[jj] + x

        def vpu_unit(t, jj):
            u, kc = divmod(t, NKC)
            stage_setup(u)
            ls = pl.ds(128 * jj, 128)
            acc = [qs_v[u, DH:DH + 8, ls]] * 2
            for d in range(DH):
                qd = jnp.broadcast_to(qs_v[u, pl.ds(d, 1), ls], (8, 128))
                for a in range(2):
                    acc[a] = acc[a] + kb_v[kc, d, pl.ds(8 * a, 8), :] * qd
            p = [jnp.exp2(x) for x in acc]
            vp[(t, jj)] = jnp.concatenate(p, axis=0)
            ladd(u, jj, p[0] + p[1])
            gval[(t, jj)] = st[u]["l"][jj]

        def pv(t):
            u, kc = divmod(t, NKC)
            vt = pltpu.bitcast(vt_v[:, pl.ds(kc * KC, KC)], _BF16)
            tiles[t][0] = jnp.concatenate([vp[(t, jj)] for jj in range(NL)], axis=1)
            pb = jnp.concatenate(tiles[t], axis=0).astype(_BF16)
            s_ = st[u]
            if t == T - 1:
                ps_v[...] = pltpu.bitcast(pb, _U32)
                po_v[...] = s_["o"]
            else:
                o = _dot(vt, pb)
                s_["o"] = o if s_["o"] is None else o + s_["o"]
            if kc == NKC - 1:
                if t < T - 1:
                    ot_v[s_["h"], :, s_["c"]] = s_["o"]
                l_v[s_["h"], :, s_["c"]] = jnp.concatenate(s_["l"], axis=1)
                for x in s_["l"]:
                    lim[0] = jnp.minimum(lim[0], x)
                    lim[1] = jnp.maximum(lim[1], x)

        def flush(group):
            if not group:
                return
            u = group[0][1] // NKC
            stage_setup(u)
            kb = []
            for i_, t, b in group:
                k_ = k_v[pl.ds((t % NKC) * (KC // 2) + 8 * b, 8), :]
                if i_ in gates:
                    pu = pltpu.bitcast(gval[gates[i_]], _U32)
                    k_ = jnp.where(never, pu[:, 0:2 * DH], k_)
                kb.append(k_)
            kk = pltpu.bitcast(jnp.concatenate(kb, axis=0), _BF16)
            s = _dot(kk, st[u]["qt"])
            for g_, (i_, t, b) in enumerate(group):
                p = jnp.exp2(s[16 * g_:16 * g_ + 16])
                a = p[0:8] + p[8:16]
                for jj in range(NL):
                    ladd(u, jj, a[:, 128 * jj:128 * jj + 128])
                tiles[t][b] = p
                for key in inserts.get(i_, []):
                    vpu_unit(*key)

        for key in inserts.get(-1, []):
            vpu_unit(*key)
        group = []
        for i_, (t, b) in enumerate(stream):
            if i_ in cuts or i_ % (7 * NKC) == 0 or len(group) >= LLAG or i_ == DPOS:
                flush(group)
                group = []
            if i_ == DPOS:
                pv_deferred(jnp.maximum(U * j - 1, 0))
            for tt in cuts.get(i_, []):
                pv(tt)
            group.append((i_, t, b))
        flush(group)
        for tt in cuts[NS]:
            pv(tt)
        return tuple(lim)

    lmin, lmax = lax.fori_loop(0, NSTAGE // U, att_body,
                               (jnp.ones((8, 128), _F32), jnp.ones((8, 128), _F32)))

    def attn_rows(r, e, pace=None):
        rows = pl.ds(pl.multiple_of(r * RB, RB), RB)
        ls = _fold8(l_v[:, :, rows])
        if pace is not None:
            never = zm_v[0:8] != 0
            ls = jnp.concatenate([jnp.concatenate(
                [jnp.where(never, pace[2 * g + i], ls[8 * g:8 * g + 8, 128 * i:128 * i + 128])
                 for i in range(RB // 128)], axis=1) for g in range(H // 8)], axis=0)
        inv_v[e] = 1.0 / ls
        o = jnp.concatenate(
            [ot_v[h, :, rows] * jnp.broadcast_to(inv_v[e, pl.ds(h, 1), :], (DH, RB))
             for h in range(H)], axis=0)
        return o.T.astype(_BF16)

    late["wmod1"].wait()
    late["wo"].wait()
    late["win"].wait()
    mod_v[:, pl.ds(2 * D, 4 * D)] = _dot(sc8, wmod_v[:, pl.ds(2 * D, 4 * D)])[0:8]
    pv_deferred(NSTAGE - 1)
    on_v[...] = pltpu.bitcast(attn_rows(0, 0), _U32)

    ok = jnp.logical_and(lmin >= L_LO, lmax <= L_HI)
    nbad = jnp.sum(jnp.where(ok, 0.0, 1.0))

    @pl.when(nbad > 0.0)
    def _():
        def slow_stage(idx, carry):
            h, c = stage_idx(idx)
            qt = jnp.concatenate([qf_v[h, :, c].astype(_BF16),
                                  jnp.zeros((DH, TQ), _BF16)], axis=0)

            def scores(kc):
                kr = pl.ds(pl.multiple_of(kc * (KC // 2), KC // 2), KC // 2)
                return _dot(pltpu.bitcast(k_v[kr, :], _BF16), qt)

            def max_body(kc, m):
                return jnp.maximum(m, jnp.max(scores(kc), axis=0, keepdims=True))

            m = lax.fori_loop(0, NKC, max_body, jnp.full((1, TQ), -jnp.inf, _F32))

            def pv_body(kc, lo):
                l, o = lo
                p = jnp.exp2(scores(kc) - m)
                ks = pl.ds(pl.multiple_of(kc * KC, KC), KC)
                vt = pltpu.bitcast(vt_v[:, ks], _BF16)
                return (l + jnp.sum(p.reshape(KC // 8, 8, TQ), axis=0),
                        o + _dot(vt, p.astype(_BF16)))

            l, o = lax.fori_loop(0, NKC, pv_body,
                                 (jnp.zeros((8, TQ), _F32), jnp.zeros((DH, TQ), _F32)))
            ot_v[h, :, c] = o
            l_v[h, :, c] = l
            return carry

        lax.fori_loop(0, NSTAGE, slow_stage, 0)
        on_v[...] = pltpu.bitcast(attn_rows(0, 0), _U32)

    def mid_a(r, e, a):
        ga = mod_v[0:1, pl.ds(2 * D, D)]
        x1 = x_v[pl.ds(pl.multiple_of((2 * r + e) * RB, RB), RB), :].astype(_F32) + ga * a
        x1_v[e][pl.ds(pl.multiple_of(r * RB, RB), RB), :] = x1
        return x1

    def mid_h(r, e, pace, step):
        sb = mod_v[0:1, pl.ds(3 * D, D)]
        cb = mod_v[0:1, pl.ds(4 * D, D)]
        x1 = x1_v[e][pl.ds(pl.multiple_of((r + zs_s[0]) * RB, RB), RB), :]
        return (paced_ln(x1, pace, step) * (1.0 + cb) + sb).astype(_BF16)

    def mid_z2(h2, e):
        zf = _gelu(_dot(h2, win_v[:, pl.ds(FH, FH)]))
        zf_v[e][0] = zf
        return zf

    def gated(w_ref, n, tiles, dep):
        never = zm_v[0:8] != 0
        du = pltpu.bitcast(dep, _U32)
        cols = []
        for c in range(n // 128):
            w = w_ref[:, pl.ds(128 * c, 128)]
            ks = [k for k, t in enumerate(tiles) if t == c]
            if ks:
                wu = pltpu.bitcast(w, _U32)
                w = pltpu.bitcast(jnp.concatenate(
                    [jnp.where(never, du[64 * (k % 2) + 56:64 * (k % 2) + 64,
                                         128 * (k // 2):128 * (k // 2) + 128],
                               wu[8 * i:8 * i + 8]) for i, k in enumerate(ks)]
                    + [wu[8 * len(ks):]], axis=0), _BF16)
            cols.append(w)
        return jnp.concatenate(cols, axis=1)

    def mid_body(r, carry):
        rows = [pl.ds(pl.multiple_of((r * 2 + e) * RB, RB), RB) for e in range(2)]
        o0 = pltpu.bitcast(on_v[...], _BF16)
        o1 = attn_rows(r * 2 + 1, 1)
        mid_a(r, 0, _dot(o0, gated(wo_v, D, OG, o1)))
        x1 = mid_a(r, 1, _dot(o1, wo_v[...]))
        h0 = mid_h(r, 0, x1, HSTEP[0])
        zf = mid_z2(h0, 0)
        h1 = mid_h(r, 1, zf, HSTEP[1])
        zf = mid_z2(h1, 1)
        z2_v[rows[0], :] = paced_ln(zf_v[0][zs_s[0]], zf, ZSTEP).astype(_BF16)
        z1 = _gelu(_dot(h0, win_v[:, pl.ds(0, FH)]))
        z1_v[rows[0], :] = z1
        z2_v[rows[1], :] = paced_ln(zf_v[1][zs_s[0]], z1, ZSTEP).astype(_BF16)
        z1 = _gelu(_dot(h1, win_v[:, pl.ds(0, FH)]))
        z1_v[rows[1], :] = z1
        pace = [divmod(OSTEP[0] + OSTEP[1] * k, RB // 16) for k in range(8)]
        pace = [z1[16 * i:16 * i + 8, 128 * j:128 * j + 128] for j, i in pace]
        on_v[...] = pltpu.bitcast(attn_rows(jnp.minimum((r + 1) * 2, NRB - 1), 0, pace), _U32)
        return carry

    lax.fori_loop(0, NRB // MU, mid_body, 0)

    late["wsp"].wait()
    late["bsp"].wait()
    late["wout"].wait()
    b32_v[...] = bsp_v[...].astype(_F32)

    def out_copy(start, n):
        rows = pl.ds(start if isinstance(start, int) else pl.multiple_of(start, n), n)
        return pltpu.make_async_copy(out_v.at[rows], o_hbm.at[0, rows], sems.at[2])

    def fin_block(j, e):
        r = 2 * j + e
        rows = pl.ds(pl.multiple_of(r * RB, RB), RB)
        gb = mod_v[0:1, pl.ds(5 * D, D)]
        bcol = jnp.concatenate(
            [jnp.broadcast_to(b32_v[pl.ds(r * (RB // 128) + i, 1), :], (128, 128)).T
             for i in range(RB // 128)], axis=0)
        g = _dot(wsp_v[rows, :], z2_v[...])
        g = g + jnp.concatenate([bcol] * (FH // 128), axis=1)
        u = (z1_v[rows, :] * g).astype(_BF16)
        n = OB[e]
        for i in range(0, RB, n):
            y = _dot(u[i:i + n], wout_v[...])
            x1 = x1_v[e][pl.ds(pl.multiple_of(j * RB + i, n), n), :]
            out_v[pl.ds(pl.multiple_of(r * RB + i, n), n), :] = (x1 + gb * y).astype(_BF16)
            out_copy(r * RB + i, n).start()

    def fin_body(j, carry):
        fin_block(j, 0)
        fin_block(j, 1)
        return carry

    lax.fori_loop(0, NRB // 2, fin_body, 0)
    for r in range(NRB):
        for i in range(0, RB, OB[r % 2]):
            out_copy(r * RB + i, OB[r % 2]).wait()


@jax.jit
def pallas_adaLN_cond__grouped_kv_mqa__mixer_gmlp__prompt_kernel(
    A_x: jax.Array,
    A_wq: jax.Array,
    A_wk: jax.Array,
    A_wv: jax.Array,
    A_wo: jax.Array,
    B_x: jax.Array,
    B_w_in: jax.Array,
    B_w_sp: jax.Array,
    B_b_sp: jax.Array,
    B_w_out: jax.Array,
    c: jax.Array,
    w_mod: jax.Array,
):
    del B_x
    any_spec = pl.BlockSpec(memory_space=pl.ANY)
    scratch = [
        pltpu.VMEM((S, D), _BF16),
        pltpu.VMEM((D, D), _BF16),
        pltpu.VMEM((2, RB // 2, D), _U32),
        pltpu.VMEM((S // 128, 128), _F32),
        pltpu.VMEM((D, D), _BF16),
        pltpu.VMEM((D, F), _BF16),
        pltpu.VMEM((S, S), _BF16),
        pltpu.VMEM((S // 128, 128), _BF16),
        pltpu.VMEM((FH, D), _BF16),
        pltpu.VMEM((1, D), _BF16),
        pltpu.VMEM((D, 6 * D), _BF16),
        pltpu.VMEM((8, 6 * D), _F32),
        pltpu.VMEM((D // 2 + DH, D), _U32),
        pltpu.VMEM((2 * DH, D), _BF16),
        pltpu.VMEM((S // 2, 2 * DH), _U32),
        pltpu.VMEM((DH // 2, S), _U32),
        pltpu.VMEM((NKC, DH, 16, 128), _F32),
        pltpu.VMEM((H, DH, S), _F32),
        pltpu.VMEM((H, S), _F32),
        pltpu.VMEM((U, DH + 8, TQ), _F32),
        pltpu.VMEM((H, 8, S), _F32),
        pltpu.VMEM((H, DH, S), _F32),
        pltpu.VMEM((8, 2 * DH), jnp.int32),
        pltpu.VMEM((S // 2, D), _F32),
        pltpu.VMEM((S // 2, D), _F32),
        pltpu.VMEM((S, FH), _F32),
        pltpu.VMEM((S, FH), _BF16),
        pltpu.VMEM((1, RB, FH), _F32),
        pltpu.VMEM((1, RB, FH), _F32),
        pltpu.VMEM((RB // 2, D), _U32),
        pltpu.VMEM((MU, H, RB), _F32),
        pltpu.VMEM((S, D), _BF16),
        pltpu.VMEM((16, 128), jnp.int32),
        pltpu.VMEM((KC // 2, TQ), _U32),
        pltpu.VMEM((DH, TQ), _F32),
        pltpu.SMEM((1,), jnp.int32),
        pltpu.SemaphoreType.DMA((5 + NRB // 2,)),
    ]
    return pl.pallas_call(
        _kernel,
        out_shape=jax.ShapeDtypeStruct((1, S, D), _BF16),
        in_specs=[any_spec] * 11,
        out_specs=any_spec,
        scratch_shapes=scratch,
        compiler_params=pltpu.CompilerParams(vmem_limit_bytes=100 * 1024 * 1024),
        name="adaln_mqa_gmlp",
    )(A_x, A_wq, A_wk.T, A_wv.T, A_wo, B_w_in, B_w_sp, B_b_sp.reshape(S // 128, 128),
      B_w_out, c, w_mod)
```
